```python
import jax
import jax.numpy as jnp

def _softmax(x, axis=-1):
    return jax.nn.softmax(x, axis=axis)
def _gelu(x):
    return jax.nn.gelu(x, approximate=True)
def _silu(x):
    return jax.nn.silu(x)
def _sigmoid(x):
    return jax.nn.sigmoid(x)
def _layernorm(x, axis=-1, eps=1e-5):
    m = jnp.mean(x, axis=axis, keepdims=True)
    v = jnp.var(x, axis=axis, keepdims=True)
    return (x - m) / jnp.sqrt(v + eps)
def _scatter_add(tgt, idx, src, axis=0):
    return tgt.at[idx].add(src)
def _segment_sum(src, seg, n):
    return jax.ops.segment_sum(src, seg, n)
class _Rng:
    def __init__(self, key):
        self._k = key
    def _next(self):
        self._k, sub = jax.random.split(self._k)
        return sub
    def normal(self, shape):
        return jax.random.normal(self._next(), shape, dtype=jnp.bfloat16)
    def randint(self, lo, hi, shape):
        return jax.random.randint(self._next(), shape, lo, hi, dtype=jnp.int32)
    def uniform(self, shape, lo=0.0, hi=1.0):
        return jax.random.uniform(self._next(), shape, jnp.bfloat16, lo, hi)
    def permutation(self, n):
        return jax.random.permutation(self._next(), n)


kernel_name = 'sequential_preLN__softmax_full_mha__glu_gated_geglu__prompt'

def _fwd_setup_inputs():
    _rng = _Rng(jax.random.key(int.from_bytes(__import__("os").urandom(4), "little")))
    _w = (lambda a: (lambda t: t.astype(jnp.bfloat16) if jnp.issubdtype(t.dtype, jnp.floating) else t)(jnp.asarray(a)))
    def _A_setup():
        B, S, D = 1, 2048, 640
        return {
            "x": _w((lambda *s: _rng.normal(s) * 0.05)(B, S, D)),
            "wqkv": _w((lambda *s: _rng.normal(s) * 0.05)(D, 3 * D)),
            "wo": _w((lambda *s: _rng.normal(s) * 0.05)(D, D)),
        }
    _A_in = _A_setup()

    def _B_setup():
        B, S, Dm, Df = 1, 2048, 640, 1536
        return {
            "x": _w((lambda *s: _rng.normal(s) * 0.05)(B, S, Dm)),
            "w_gate": _w((lambda *s: _rng.normal(s) * 0.05)(Dm, Df) * (Dm ** -0.5)),
            "w_up": _w((lambda *s: _rng.normal(s) * 0.05)(Dm, Df) * (Dm ** -0.5)),
            "w_down": _w((lambda *s: _rng.normal(s) * 0.05)(Df, Dm) * (Df ** -0.5)),
        }
    _B_in = _B_setup()

    return {
        "A_x": _A_in["x"],
        "A_wqkv": _A_in["wqkv"],
        "A_wo": _A_in["wo"],
        "B_x": _B_in["x"],
        "B_w_gate": _B_in["w_gate"],
        "B_w_up": _B_in["w_up"],
        "B_w_down": _B_in["w_down"],
    }

def _fwd_reference(A_x, A_wqkv, A_wo, B_x, B_w_gate, B_w_up, B_w_down):
    def _A_ref(x, wqkv, wo):
        B, S, D = x.shape
        H = 32; Dh = D // H
        qkv = (lambda x, *d: x.transpose(*d))((x @ wqkv).reshape(B, S, 3, H, Dh), 2, 0, 3, 1, 4)
        q, k, v = qkv[0], qkv[1], qkv[2]
        scale = Dh ** -0.5
        scores = jnp.einsum("bhqd,bhkd->bhqk", q, k) * scale
        p = _softmax(scores, axis=-1)
        o = jnp.einsum("bhqk,bhkd->bhqd", p, v)
        return (lambda x, *d: x.transpose(*d))(o, 0, 2, 1, 3).reshape(B, S, D) @ wo

    def _B_ref(x, w_gate, w_up, w_down):
        g = jnp.einsum("bsd,df->bsf", x, w_gate)
        u = jnp.einsum("bsd,df->bsf", x, w_up)
        h = _gelu(g) * u
        return jnp.einsum("bsf,fd->bsd", h, w_down)

    x = A_x
    h = x + _A_ref(_layernorm(x, axis=-1), A_wqkv, A_wo)
    h2 = h + _B_ref(_layernorm(h, axis=-1), B_w_gate, B_w_up, B_w_down)
    return h2


def setup_inputs():
    _inp = _fwd_setup_inputs()
    _gk = jax.random.fold_in(jax.random.key(int.from_bytes(__import__("os").urandom(4), "little")), 2**31 - 1)
    _shapes = [[1, 2048, 640]]
    _dtypes = ['bfloat16']
    _gks = jax.random.split(_gk, len(_shapes))
    _gs = [jax.random.normal(k, s, dtype=jnp.dtype(d)) * 0.05 for k, s, d in zip(_gks, _shapes, _dtypes)]
    _inp["grad_out"] = _gs[0]
    return _inp

def reference(A_x, A_wqkv, A_wo, B_w_gate, B_w_up, B_w_down, B_x, grad_out):
    _const = dict(B_x=B_x)
    def _f(*_d):
        return _fwd_reference(**{'A_x': _d[0], 'A_wqkv': _d[1], 'A_wo': _d[2], 'B_w_gate': _d[3], 'B_w_up': _d[4], 'B_w_down': _d[5], **_const})
    _out, _vjp = jax.vjp(_f, A_x, A_wqkv, A_wo, B_w_gate, B_w_up, B_w_down)
    _grads = _vjp(grad_out)
    _out0 = jnp.asarray(_out)
    return (_out0, *[jnp.asarray(_g) for _g in _grads])
```

```python
import math

import jax
import jax.numpy as jnp
import jax.experimental.pallas as pl
import jax.experimental.pallas.tpu as pltpu

f32 = jnp.float32
bf16 = jnp.bfloat16
u32 = jnp.uint32

S = 2048
D = 640
H = 32
DH = 20
DF = 1536
TQ = 256
NB = S // TQ
FC = 256
NFC = DF // FC
NG = 6
CK = 256
SUB = 128
NCK = S // CK
WC = 384
NWC = 3 * D // WC
EPS = 1e-5
SCALE = DH ** -0.5
QSCALE = SCALE * math.log2(math.e)
LN2 = math.log(2.0)
GELU_C = math.sqrt(2.0 / math.pi)
GELU_A = 0.044715

NT = (((1,), (1,)), ((), ()))


def _group_col(g):
    return 120 * g if g < 5 else 512


def _dot(a, b):
    return jnp.dot(a, b, preferred_element_type=f32)


def _dot_nt(a, b):
    return jax.lax.dot_general(a, b, NT, preferred_element_type=f32)


def _pk(x):
    return pltpu.bitcast(x.astype(bf16), u32)


def _upk(x):
    return pltpu.bitcast(x, bf16)


def _layernorm(x):
    mu = jnp.mean(x, axis=-1, keepdims=True)
    xc = x - mu
    var = jnp.mean(xc * xc, axis=-1, keepdims=True)
    rstd = jax.lax.rsqrt(var + EPS)
    return xc * rstd, rstd


def _layernorm_bwd(dy, y, rstd):
    m1 = jnp.mean(dy, axis=-1, keepdims=True)
    m2 = jnp.mean(dy * y, axis=-1, keepdims=True)
    return rstd * (dy - m1 - y * m2)


def _head_scalars(h):
    g = jax.lax.shift_right_logical(h * 43, 8)
    cg = jnp.where(g < 5, g * 120, 512)
    ro = DH * h - cg
    wg = jax.lax.shift_right_logical(ro, 4) * 16
    ws = jax.lax.shift_right_logical(DH * h, 3) * 8
    return g, cg, ro, wg, ws


def _row_mask(nrows, lo):
    r = jax.lax.broadcasted_iota(jnp.int32, (nrows, TQ), 0)
    return jnp.logical_and(r >= lo, r < lo + DH)


def _kernel(x_hbm, wqkv_hbm, wo_hbm, wg_hbm, wu_hbm, wd_hbm, gy_hbm,
            h2_hbm, dx_hbm, dwqkv_hbm, dwo_hbm, dwg_hbm, dwu_hbm, dwd_hbm,
            x_v, gy_v, wqkv_v, wo_v, wg_v, wu_v, wd_v, h2_v,
            qt, knat, vnat, ktg, vaug, xnt, dkt, dvt, dqt, dh_v,
            a_wg, a_wu, a_wd, a_wo,
            sem_x, sem_in, sem_h2, sem_dx, sem_w, sem_wq):

    def x_copy(b):
        return pltpu.make_async_copy(x_hbm.at[pl.ds(b * TQ, TQ), :],
                                     x_v.at[pl.ds(b * TQ, TQ), :], sem_x.at[b])

    in_copies = [pltpu.make_async_copy(wqkv_hbm, wqkv_v, sem_in.at[0]),
                 pltpu.make_async_copy(wo_hbm, wo_v, sem_in.at[1]),
                 pltpu.make_async_copy(gy_hbm, gy_v, sem_in.at[2])]
    for c in range(NFC):
        cs = pl.ds(c * FC, FC)
        in_copies.append(pltpu.make_async_copy(wg_hbm.at[:, cs], wg_v.at[c], sem_in.at[3 + 3 * c]))
        in_copies.append(pltpu.make_async_copy(wu_hbm.at[:, cs], wu_v.at[c], sem_in.at[4 + 3 * c]))
        in_copies.append(pltpu.make_async_copy(wd_hbm.at[cs, :], wd_v.at[c], sem_in.at[5 + 3 * c]))

    in_copies[0].start()
    for b in range(NB):
        x_copy(b).start()
    for cp in in_copies[1:]:
        cp.start()

    dkt[...] = jnp.zeros_like(dkt)
    dvt[...] = jnp.zeros_like(dvt)
    a_wg[...] = jnp.zeros_like(a_wg)
    a_wu[...] = jnp.zeros_like(a_wu)
    a_wd[...] = jnp.zeros_like(a_wd)
    a_wo[...] = jnp.zeros_like(a_wo)

    def phase0(wgrp):
        in_copies[0].wait()
        for t in range(2):
            for g in range(NG):
                c0 = (t + 1) * D + _group_col(g)
                wgrp[t * NG + g] = wqkv_v[:, c0:c0 + 128]

        def blk(b, carry):
            pltpu.make_async_copy(x_hbm.at[pl.ds(0, TQ), :], x_v.at[pl.ds(0, TQ), :],
                                  sem_x.at[b]).wait()
            r0 = pl.multiple_of(b * TQ, TQ)
            r2 = pl.multiple_of(b * (TQ // 2), TQ // 2)
            xn, _ = _layernorm(x_v[pl.ds(r0, TQ), :].astype(f32))
            xb = xn.astype(bf16)
            xnt[:, pl.ds(r0, TQ)] = _pk(xn.T)
            q = _dot(xb, wqkv_v[:, 0:D]) * QSCALE
            qt[b] = q.T
            rows = jax.lax.broadcasted_iota(jnp.int32, (32, TQ), 0)
            for g in range(NG):
                k = _dot(xb, wgrp[g])
                knat[g, pl.ds(r2, TQ // 2), :] = _pk(k)
                ktg[g, :, pl.ds(r0, TQ)] = _pk(k.T)
                v = _dot(xb, wgrp[NG + g])
                vnat[g, pl.ds(r2, TQ // 2), :] = _pk(v)
                vt = v.T
                for h in range(6 * g, min(6 * g + 6, H)):
                    ro = DH * h - _group_col(g)
                    wg0 = (ro // 16) * 16
                    one_row = 31 if ro - wg0 < 12 else 0
                    win = jnp.where(rows == one_row, 1.0, vt[wg0:wg0 + 32])
                    vaug[h, :, pl.ds(r0, TQ)] = _pk(win)
            return carry

        jax.lax.fori_loop(0, NB, blk, 0)

    pl.run_scoped(phase0, pltpu.VMEM((2 * NG, D, 128), bf16))

    for cp in in_copies[1:]:
        cp.wait()

    def main(p_scr, sa, sb, ma, mb, ot, dot_, dqb, linv, hn_f, hn_b, hnt, dyt, otb,
             y_acc, dhn_acc, rstd_v):
        ot[...] = jnp.zeros_like(ot)
        dqb[...] = jnp.zeros_like(dqb)

        def qblock(qb, carry):
            r0 = pl.multiple_of(qb * TQ, TQ)
            z = jax.lax.shift_right_logical(qb, 20) * 8

            def wq_of(h):
                g, cg, ro, _, _ = _head_scalars(h)
                qg = qt[qb, pl.ds(pl.multiple_of(cg, 8), 128), :]
                return g, jnp.where(_row_mask(128, ro), qg, 0.0).astype(bf16)

            def fwd_stage(h, hn, s_cur, m_cur, s_nxt, m_nxt):
                if hn is not None:
                    g, w = wq_of(hn)
                if h is not None:
                    mrow = m_cur[0:1, :]
                m = None
                o = None
                for c in range(NCK):
                    if hn is not None:
                        for s0 in range(0, CK, SUB):
                            r = c * CK + s0
                            s = _dot(_upk(knat[g, pl.ds(r // 2, SUB // 2), :]), w)
                            s_nxt[pl.ds(r, SUB), :] = s
                            mc = jnp.max(s.reshape(SUB // 8, 8, TQ), axis=0)
                            m = mc if m is None else jnp.maximum(m, mc)
                    if h is not None:
                        sv = s_cur[pl.ds(pl.multiple_of(z + c * CK, 8), CK), :]
                        pk = _pk(jnp.exp2(sv - mrow))
                        p_scr[h, pl.ds(c * CK // 2, CK // 2), :] = pk
                        oc = _dot(_upk(vaug[h, :, pl.ds(c * CK, CK)]), _upk(pk))
                        o = oc if o is None else o + oc
                if hn is not None:
                    m_nxt[...] = jnp.broadcast_to(jnp.max(m, axis=0, keepdims=True), (8, TQ))
                if h is not None:
                    _, cg, ro, wg, _ = _head_scalars(h)
                    off = ro - wg
                    l = jnp.where(off < 12, o[31:32], o[0:1])
                    li = 1.0 / l
                    linv[h] = jnp.broadcast_to(li, (8, TQ))
                    rs = pl.ds(pl.multiple_of(cg + wg, 8), 32)
                    ot[rs, :] = jnp.where(_row_mask(32, off), o * li, ot[rs, :])

            fwd_stage(None, 0, None, None, sa, ma)

            def fwd_pair(i, c):
                h0 = 2 * i
                fwd_stage(h0, h0 + 1, sa, ma, sb, mb)
                fwd_stage(h0 + 1, h0 + 2, sb, mb, sa, ma)
                return c

            jax.lax.fori_loop(0, H // 2 - 1, fwd_pair, 0)
            fwd_stage(H - 2, H - 1, sa, ma, sb, mb)
            fwd_stage(H - 1, None, sb, mb, None, None)

            o_t = ot[...]
            otb[...] = _pk(o_t)
            attn = _dot(o_t.T.astype(bf16), wo_v[...])
            hres = x_v[pl.ds(r0, TQ), :].astype(f32) + attn
            y_acc[...] = hres
            hn, rstd = _layernorm(hres)
            hn_f[...] = hn
            rstd_v[...] = rstd
            hn_b[...] = _pk(hn)
            hnt[...] = _pk(hn.T)
            dyt[...] = _pk(gy_v[pl.ds(r0, TQ), :].astype(f32).T)
            dhn_acc[...] = jnp.zeros_like(dhn_acc)

            def ffn_a(c):
                hb = _upk(hn_b[...])
                g = _dot(hb, wg_v[c])
                u = _dot(hb, wu_v[c])
                da = _dot_nt(gy_v[pl.ds(r0, TQ), :], wd_v[c])
                return g, u, da

            def ffn_b(c, g, u, da):
                g2 = g * g
                t = jnp.tanh(GELU_C * g * (1.0 + GELU_A * g2))
                hg = 0.5 * g
                gel = hg + hg * t
                dgel = 0.5 + 0.5 * t + hg * (1.0 - t * t) * (GELU_C + 3.0 * GELU_A * GELU_C * g2)
                a = (gel * u).astype(bf16)
                dg = (da * u * dgel).astype(bf16)
                du = (da * gel).astype(bf16)
                y_acc[...] += _dot(a, wd_v[c])
                dhn_acc[...] += _dot_nt(dg, wg_v[c]) + _dot_nt(du, wu_v[c])
                ht = _upk(hnt[...])
                a_wg[c] += _dot(ht, dg)
                a_wu[c] += _dot(ht, du)
                a_wd[c] += _dot(_upk(dyt[...]), a)

            def ffn_pair(i, c):
                r_0 = ffn_a(2 * i)
                r_1 = ffn_a(2 * i + 1)
                ffn_b(2 * i, *r_0)
                ffn_b(2 * i + 1, *r_1)
                return c

            jax.lax.fori_loop(0, NFC // 2, ffn_pair, 0)

            h2_v[pl.ds(r0, TQ), :] = y_acc[...].astype(bf16)
            pltpu.make_async_copy(h2_v.at[pl.ds(r0, TQ), :], h2_hbm.at[pl.ds(r0, TQ), :],
                                  sem_h2.at[qb]).start()

            dh = gy_v[pl.ds(r0, TQ), :].astype(f32) + _layernorm_bwd(
                dhn_acc[...], hn_f[...], rstd_v[...])
            dh_v[pl.ds(r0, TQ), :] = dh
            dhb = dh.astype(bf16)
            dot_[...] = _dot_nt(wo_v[...], dhb)
            a_wo[...] += _dot(_upk(otb[...]), dhb)

            def bwd_heads(i, carry2, hpi):
                hs = [hpi * i + k for k in range(hpi)]
                pre = []
                for h in hs:
                    g, cg, ro, wg, ws = _head_scalars(h)
                    li = linv[h][0:1, :]
                    dg_ = dot_[pl.ds(pl.multiple_of(cg, 8), 128), :]
                    w = jnp.where(_row_mask(128, ro), dg_ * li, 0.0).astype(bf16)
                    rs = pl.ds(pl.multiple_of(ws, 8), 24)
                    m24 = _row_mask(24, DH * h - ws)
                    dos = jnp.where(m24, dot_[rs, :] * li, 0.0)
                    delta = jnp.sum(dos * ot[rs, :], axis=0, keepdims=True)
                    zeros8 = jnp.zeros((8, TQ), f32)
                    do_l = jnp.concatenate([dos, zeros8], axis=0).astype(bf16)
                    q_l = jnp.concatenate(
                        [jnp.where(m24, qt[qb, rs, :], 0.0), zeros8], axis=0).astype(bf16)
                    pre.append((g, cg, ro, wg, rs, w, delta, do_l, q_l))

                steps = [(k, c) for k in range(hpi) for c in range(NCK)]

                def dp_of(k, c):
                    g, w = pre[k][0], pre[k][5]
                    parts = []
                    for s0 in range(0, CK, SUB):
                        r = c * CK + s0
                        parts.append(_dot(_upk(vnat[g, pl.ds(r // 2, SUB // 2), :]), w))
                    return jnp.concatenate(parts, axis=0)

                dp = dp_of(*steps[0])
                dq = None
                for n, (k, c) in enumerate(steps):
                    h = hs[k]
                    g, cg, ro, wg, rs, w, delta, do_l, q_l = pre[k]
                    dp_next = dp_of(*steps[n + 1]) if n + 1 < len(steps) else None
                    sl = pl.ds(c * CK, CK)
                    p = _upk(p_scr[h, pl.ds(c * CK // 2, CK // 2), :])
                    ds = (p.astype(f32) * (dp - delta)).astype(bf16)
                    dvt[rs, sl] += _dot_nt(do_l, p)[0:24]
                    dkt[rs, sl] += _dot_nt(q_l, ds)[0:24]
                    kt = _upk(ktg[g, pl.ds(pl.multiple_of(wg // 2, 8), 16), sl])
                    dqc = _dot(kt, ds)
                    dq = dqc if c == 0 else dq + dqc
                    if c == NCK - 1:
                        rq = pl.ds(pl.multiple_of(cg + wg, 8), 32)
                        dqb[rq, :] = jnp.where(_row_mask(32, ro - wg), dq * SCALE, dqb[rq, :])
                    dp = dp_next
                return carry2

            jax.lax.fori_loop(0, H // 2, lambda i, c: bwd_heads(i, c, 2), 0)
            dqt[qb] = _pk(dqb[...])
            return carry

        jax.lax.fori_loop(0, NB, qblock, 0)

    pl.run_scoped(
        main,
        pltpu.VMEM((H, S // 2, TQ), u32),
        pltpu.VMEM((S, TQ), f32),
        pltpu.VMEM((S, TQ), f32),
        pltpu.VMEM((8, TQ), f32),
        pltpu.VMEM((8, TQ), f32),
        pltpu.VMEM((D, TQ), f32),
        pltpu.VMEM((D, TQ), f32),
        pltpu.VMEM((D, TQ), f32),
        pltpu.VMEM((H, 8, TQ), f32),
        pltpu.VMEM((TQ, D), f32),
        pltpu.VMEM((TQ // 2, D), u32),
        pltpu.VMEM((D // 2, TQ), u32),
        pltpu.VMEM((D // 2, TQ), u32),
        pltpu.VMEM((D // 2, TQ), u32),
        pltpu.VMEM((TQ, D), f32),
        pltpu.VMEM((TQ, D), f32),
        pltpu.VMEM((TQ, 1), f32),
    )

    w_copies = [pltpu.make_async_copy(wo_v, dwo_hbm, sem_w.at[0])]
    wo_v[...] = a_wo[...].astype(bf16)
    w_copies[0].start()
    for c in range(NFC):
        cs = pl.ds(c * FC, FC)
        wg_v[c] = a_wg[c].astype(bf16)
        wu_v[c] = a_wu[c].astype(bf16)
        wd_v[c] = a_wd[c].T.astype(bf16)
        new = [pltpu.make_async_copy(wg_v.at[c], dwg_hbm.at[:, cs], sem_w.at[1 + 3 * c]),
               pltpu.make_async_copy(wu_v.at[c], dwu_hbm.at[:, cs], sem_w.at[2 + 3 * c]),
               pltpu.make_async_copy(wd_v.at[c], dwd_hbm.at[cs, :], sem_w.at[3 + 3 * c])]
        for cp in new:
            cp.start()
        w_copies += new

    def phase2(dqkvt, dw_st):
        def blk(b, carry):
            r0 = pl.multiple_of(b * TQ, TQ)
            cs = pl.ds(r0, TQ)
            dqkvt[0:D // 2, cs] = dqt[b]
            dqkvt[D // 2:D, cs] = _pk(dkt[:, cs] * LN2)
            dqkvt[D:3 * D // 2, cs] = _pk(dvt[:, cs])
            dxnt = _dot(wqkv_v[...], _upk(dqkvt[:, cs]))
            xn, rstd = _layernorm(x_v[cs, :].astype(f32))
            dx = dh_v[cs, :] + _layernorm_bwd(dxnt.T, xn, rstd)
            gy_v[cs, :] = dx.astype(bf16)
            pltpu.make_async_copy(gy_v.at[cs, :], dx_hbm.at[cs, :], sem_dx.at[b]).start()
            return carry

        jax.lax.fori_loop(0, NB, blk, 0)

        def wchunk(n, carry):
            rr = pl.ds(pl.multiple_of(n * (WC // 2), 8), WC // 2)
            dw_st[n] = _dot_nt(_upk(xnt[...]), _upk(dqkvt[rr, :])).astype(bf16)
            pltpu.make_async_copy(
                dw_st.at[n], dwqkv_hbm.at[:, pl.ds(pl.multiple_of(n * WC, 128), WC)],
                sem_wq.at[n]).start()
            return carry

        jax.lax.fori_loop(0, NWC, wchunk, 0)
        for n in range(NWC):
            pltpu.make_async_copy(dw_st.at[n], dwqkv_hbm.at[:, pl.ds(n * WC, WC)],
                                  sem_wq.at[n]).wait()

    pl.run_scoped(phase2,
                  pltpu.VMEM((3 * D // 2, S), u32),
                  pltpu.VMEM((NWC, D, WC), bf16))

    for b in range(NB):
        rs = pl.ds(b * TQ, TQ)
        pltpu.make_async_copy(h2_v.at[rs, :], h2_hbm.at[rs, :], sem_h2.at[b]).wait()
        pltpu.make_async_copy(gy_v.at[rs, :], dx_hbm.at[rs, :], sem_dx.at[b]).wait()
    for cp in w_copies:
        cp.wait()


@jax.jit
def pallas_sequential_preLN__softmax_full_mha__glu_gated_geglu__prompt_kernel(
    A_x: jax.Array,
    A_wqkv: jax.Array,
    A_wo: jax.Array,
    B_x: jax.Array,
    B_w_gate: jax.Array,
    B_w_up: jax.Array,
    B_w_down: jax.Array,
    grad_out: jax.Array,
):
    del B_x
    any_spec = pl.BlockSpec(memory_space=pl.ANY)
    out_shape = (
        jax.ShapeDtypeStruct((S, D), bf16),
        jax.ShapeDtypeStruct((S, D), bf16),
        jax.ShapeDtypeStruct((D, 3 * D), bf16),
        jax.ShapeDtypeStruct((D, D), bf16),
        jax.ShapeDtypeStruct((D, DF), bf16),
        jax.ShapeDtypeStruct((D, DF), bf16),
        jax.ShapeDtypeStruct((DF, D), bf16),
    )
    scratch = [
        pltpu.VMEM((S, D), bf16),
        pltpu.VMEM((S, D), bf16),
        pltpu.VMEM((D, 3 * D), bf16),
        pltpu.VMEM((D, D), bf16),
        pltpu.VMEM((NFC, D, FC), bf16),
        pltpu.VMEM((NFC, D, FC), bf16),
        pltpu.VMEM((NFC, FC, D), bf16),
        pltpu.VMEM((S, D), bf16),
        pltpu.VMEM((NB, D, TQ), f32),
        pltpu.VMEM((NG, S // 2, 128), u32),
        pltpu.VMEM((NG, S // 2, 128), u32),
        pltpu.VMEM((NG, 64, S), u32),
        pltpu.VMEM((H, 16, S), u32),
        pltpu.VMEM((D // 2, S), u32),
        pltpu.VMEM((D, S), f32),
        pltpu.VMEM((D, S), f32),
        pltpu.VMEM((NB, D // 2, TQ), u32),
        pltpu.VMEM((S, D), f32),
        pltpu.VMEM((NFC, D, FC), f32),
        pltpu.VMEM((NFC, D, FC), f32),
        pltpu.VMEM((NFC, D, FC), f32),
        pltpu.VMEM((D, D), f32),
        pltpu.SemaphoreType.DMA((NB,)),
        pltpu.SemaphoreType.DMA((3 + 3 * NFC,)),
        pltpu.SemaphoreType.DMA((NB,)),
        pltpu.SemaphoreType.DMA((NB,)),
        pltpu.SemaphoreType.DMA((1 + 3 * NFC,)),
        pltpu.SemaphoreType.DMA((NWC,)),
    ]
    outs = pl.pallas_call(
        _kernel,
        out_shape=out_shape,
        in_specs=[any_spec] * 7,
        out_specs=[any_spec] * 7,
        scratch_shapes=scratch,
        compiler_params=pltpu.CompilerParams(vmem_limit_bytes=124 * 1024 * 1024),
    )(A_x.reshape(S, D), A_wqkv, A_wo, B_w_gate, B_w_up, B_w_down, grad_out.reshape(S, D))
    h2, dx, dwqkv, dwo, dwg, dwu, dwd = outs
    return (h2.reshape(1, S, D), dx.reshape(1, S, D), dwqkv, dwo, dwg, dwu, dwd)
```

```python
import math

import jax
import jax.numpy as jnp
import jax.experimental.pallas as pl
import jax.experimental.pallas.tpu as pltpu

f32 = jnp.float32
bf16 = jnp.bfloat16
u32 = jnp.uint32

S = 2048
D = 640
H = 32
DH = 20
DF = 1536
TQ = 256
NB = S // TQ
FC = 256
NFC = DF // FC
NG = 6
CK = 256
SUB = 128
NCK = S // CK
WC = 128
EPS = 1e-5
SCALE = DH ** -0.5
QSCALE = SCALE * math.log2(math.e)
LN2 = math.log(2.0)
GELU_C = math.sqrt(2.0 / math.pi)
GELU_A = 0.044715

NN = (((1,), (0,)), ((), ()))
NT = (((1,), (1,)), ((), ()))
HPF = 8
HPB = 8
NP = NCK
NS = 2
ZB = 5
LAG = 1


def _group_col(g):
    return 120 * g if g < 5 else 512


def _dot(a, b):
    return jax.lax.dot_general(a, b, NN, preferred_element_type=f32)


def _dot_nt(a, b):
    return jax.lax.dot_general(a, b, NT, preferred_element_type=f32)


def _pk(x):
    return pltpu.bitcast(x.astype(bf16), u32)


def _upk(x):
    return pltpu.bitcast(x, bf16)


def _prow(i, start, size):
    return pl.ds(pl.multiple_of(i * (S // 2) + start, 8), size)


def _pslot(h, z=0):
    return pl.ds(pl.multiple_of(z + h * (CK // 2), 8), CK // 2)


def _layernorm(x):
    mu = jnp.mean(x, axis=-1, keepdims=True)
    xc = x - mu
    var = jnp.mean(xc * xc, axis=-1, keepdims=True)
    rstd = jax.lax.rsqrt(var + EPS)
    return xc * rstd, rstd


def _layernorm_bwd(dy, y, rstd):
    m1 = jnp.mean(dy, axis=-1, keepdims=True)
    m2 = jnp.mean(dy * y, axis=-1, keepdims=True)
    return rstd * (dy - m1 - y * m2)


def _head_scalars(h):
    g = jax.lax.shift_right_logical(h * 43, 8)
    cg = jnp.where(g < 5, g * 120, 512)
    ro = DH * h - cg
    ws = jax.lax.shift_right_logical(DH * h, 3) * 8
    return g, cg, ro, ws, DH * h - ws


def _row_mask(nrows, lo):
    r = jax.lax.broadcasted_iota(jnp.int32, (nrows, TQ), 0)
    return jnp.logical_and(r >= lo, r < lo + DH)


def _kernel(x_hbm, wqkv_hbm, wo_hbm, wg_hbm, wu_hbm, wd_hbm, gy_hbm,
            h2_hbm, dx_hbm, dwqkv_hbm, dwo_hbm, dwg_hbm, dwu_hbm, dwd_hbm,
            x_v, gy_v, wqkv_v, wo_v, wg_v, wu_v, wd_v, h2_v,
            qt, knat, vnat, kt, vt, xnt, dkt, dvt, dqt, dh_v,
            a_wg, a_wu, a_wd, a_wo,
            p_refs, s_a, s_b, m_v, ot, dot_, dqb, linv, hn_f, hn_b, hnt,
            otb, y_acc, dhn_acc, rstd_v, da_v, ds0,
            sem_x, sem_qkv, sem_in, sem_h2, sem_dx, sem_w, sem_wq):

    def x_copy(b):
        rs = pl.ds(pl.multiple_of(b * TQ, TQ), TQ)
        return pltpu.make_async_copy(x_hbm.at[rs, :], x_v.at[rs, :], sem_x.at[b])

    qkv_copies = [pltpu.make_async_copy(wqkv_hbm.at[:, pl.ds(t * D, D)],
                                        wqkv_v.at[:, pl.ds(t * D, D)], sem_qkv.at[t])
                  for t in range(3)]
    in_copies = [pltpu.make_async_copy(wo_hbm, wo_v, sem_in.at[0]),
                 pltpu.make_async_copy(gy_hbm, gy_v, sem_in.at[1])]
    for c in range(NFC):
        cs = pl.ds(c * FC, FC)
        in_copies.append(pltpu.make_async_copy(wg_hbm.at[:, cs], wg_v.at[c], sem_in.at[2 + 3 * c]))
        in_copies.append(pltpu.make_async_copy(wu_hbm.at[:, cs], wu_v.at[c], sem_in.at[3 + 3 * c]))
        in_copies.append(pltpu.make_async_copy(wd_hbm.at[cs, :], wd_v.at[c], sem_in.at[4 + 3 * c]))

    x_copy(0).start()
    qkv_copies[1].start()

    def zero_blk(b, carry):
        cs = pl.ds(pl.multiple_of(b * TQ, TQ), TQ)
        dkt[:, cs] = jnp.zeros((D, TQ), f32)
        dvt[:, cs] = jnp.zeros((D, TQ), f32)
        return carry

    jax.lax.fori_loop(0, ZB, zero_blk, 0)
    qkv_copies[2].start()
    x_copy(1).start()
    jax.lax.fori_loop(ZB, NB, zero_blk, 0)

    def ln_block(b):
        r0 = pl.multiple_of(b * TQ, TQ)
        xn, _ = _layernorm(x_v[pl.ds(r0, TQ), :].astype(f32))
        xnt[:, pl.ds(r0, TQ)] = _pk(xn.T)
        return _pk(xn)

    def proj_block(b, xb_p, first):
        r0 = pl.multiple_of(b * TQ, TQ)
        r2 = pl.multiple_of(b * (TQ // 2), TQ // 2)
        xb = _upk(xb_p)

        def finish(y, nat, tr):
            y_t = y.T
            tr[:, pl.ds(r0, TQ)] = y_t
            for g in range(NG):
                c0 = _group_col(g)
                nat[_prow(g, r2, TQ // 2), :] = _pk(y_t[c0:c0 + 128].T)

        if first:
            qkv_copies[1].wait()
            qkv_copies[0].start()
        k = _dot(xb, wqkv_v[:, D:2 * D])
        if first:
            qkv_copies[2].wait()
            x_copy(1).wait()
            v = _dot(xb, wqkv_v[:, 2 * D:3 * D])
            finish(k, knat, kt)
            for bb in range(2, NB):
                x_copy(bb).start()
            qkv_copies[0].wait()
            q = _dot(xb, wqkv_v[:, 0:D]) * QSCALE
            xb_next = ln_block(1)
            finish(v, vnat, vt)
        else:
            xb_next = ln_block(jnp.minimum(b + 1, NB - 1))
            finish(k, knat, kt)
            finish(_dot(xb, wqkv_v[:, 2 * D:3 * D]), vnat, vt)
            q = _dot(xb, wqkv_v[:, 0:D]) * QSCALE
        qt[b] = q.T
        return xb_next

    def phase0():
        x_copy(0).wait()
        xb1 = proj_block(0, ln_block(0), True)

        def blk(b, xb_p):
            @pl.when(b == 2)
            def _():
                for cp in in_copies:
                    cp.start()

            @pl.when(b + 1 < NB)
            def _():
                x_copy(b + 1).wait()

            return proj_block(b, xb_p, False)

        jax.lax.fori_loop(1, NB, blk, xb1)

    phase0()

    for cp in in_copies:
        cp.wait()

    def main():
        ot[...] = jnp.zeros_like(ot)
        dqb[...] = jnp.zeros_like(dqb)
        sbuf = (s_a, s_b)
        HC = NCK // NS

        def save_dq(b):
            dqt[pl.ds(pl.multiple_of(b * (D // 2), 8), D // 2), :] = _pk(dqb[...])

        def score_weights(qn, hn):
            g, cg, ro, _, _ = _head_scalars(hn)
            qg = qt[qn, pl.ds(pl.multiple_of(cg, 8), 128), :]
            return g, jnp.where(_row_mask(128, ro), qg, 0.0).astype(bf16)

        def score_chunk(g, w, c, dst, m):
            for s0 in range(0, CK, SUB):
                r = c * CK + s0
                s = _dot(_upk(knat[_prow(g, r // 2, SUB // 2), :]), w)
                dst[c // HC][pl.ds((c % HC) * CK + s0, SUB), :] = s
                mc = jnp.max(s.reshape(SUB // 8, 8, TQ), axis=0)
                m = mc if m is None else jnp.maximum(m, mc)
            return m

        g0, w0 = score_weights(0, 0)
        m0 = None
        for c in range(NCK):
            m0 = score_chunk(g0, w0, c, sbuf[0], m0)
        m_v[...] = jnp.broadcast_to(jnp.max(m0, axis=0, keepdims=True), (8, TQ))
        da_v[0] = _dot_nt(gy_v[0:TQ, :], wd_v[0])

        def qblock(qb, carry):
            r0 = pl.multiple_of(qb * TQ, TQ)
            z = jax.lax.shift_right_logical(qb, 20) * 8
            later = qb > 0

            def acc(old, new):
                return jnp.where(later, old, 0.0) + new

            def fwd_iter(i, carry2):
                hs = [HPF * i + k for k in range(HPF)]
                wrap = jax.lax.shift_right_logical(hs[-1] + 1, 5)
                nxt = [(qb, h + 1) for h in hs[:-1]]
                nxt.append((jnp.minimum(qb + wrap, NB - 1), jnp.bitwise_and(hs[-1] + 1, H - 1)))
                mrow = [m_v[0:1, :]]
                rows = jax.lax.broadcasted_iota(jnp.int32, (24, CK), 0)
                n_steps = HPF * NCK
                m = o = gw = None
                for n in range(n_steps + LAG):
                    if n < n_steps:
                        k, c = divmod(n, NCK)
                        if c == 0:
                            gw = score_weights(*nxt[k])
                            m = None
                        m = score_chunk(gw[0], gw[1], c, sbuf[(k + 1) % 2], m)
                        if c == NCK - 1:
                            mrow.append(jnp.max(m, axis=0, keepdims=True))
                    if n >= LAG:
                        k, c = divmod(n - LAG, NCK)
                        h = hs[k]
                        _, _, _, ws, off = _head_scalars(h)
                        rs = pl.ds(pl.multiple_of(ws, 8), 24)
                        src = sbuf[k % 2][c // HC]
                        sv = src[pl.ds(pl.multiple_of(z + (c % HC) * CK, 8), CK), :]
                        p = jnp.exp2(sv - mrow[k]).astype(bf16)
                        p_refs[c][_pslot(h), :] = pltpu.bitcast(p, u32)
                        ones_row = rows == jnp.where(off == 0, 23, 0)
                        vl = jnp.where(ones_row, 1.0, vt[rs, pl.ds(c * CK, CK)])
                        oc = _dot(vl, p)
                        o = oc if c == 0 else o + oc
                        if c == NCK - 1:
                            l = jnp.where(off == 0, o[23:24], o[0:1])
                            li = 1.0 / l
                            linv[h] = jnp.broadcast_to(li, (8, TQ))
                            ot[rs, :] = jnp.where(_row_mask(24, off), o * li, ot[rs, :])
                m_v[...] = jnp.broadcast_to(mrow[-1], (8, TQ))
                return carry2

            jax.lax.fori_loop(0, H // HPF, fwd_iter, 0)

            gyb = gy_v[pl.ds(r0, TQ), :]
            da_v[1] = _dot_nt(gyb, wd_v[1])
            save_dq(jnp.maximum(qb - 1, 0))
            o_t = ot[...]
            otb[...] = _pk(o_t)
            attn = _dot(o_t.T.astype(bf16), wo_v[...])
            for c in range(2, NFC):
                da_v[c] = _dot_nt(gyb, wd_v[c])
            hres = x_v[pl.ds(r0, TQ), :].astype(f32) + attn
            y_acc[...] = hres
            hn, rstd = _layernorm(hres)
            hn_f[...] = hn
            rstd_v[...] = rstd
            hn_b[...] = _pk(hn)
            hnt[...] = _pk(hn.T)
            dhn_acc[...] = jnp.zeros_like(dhn_acc)

            def ffn_a(c):
                hb = _upk(hn_b[...])
                g = _dot(hb, wg_v[c])
                u = _dot(hb, wu_v[c])
                return g, u

            def ffn_b(c, g, u):
                da = da_v[c]
                g2 = g * g
                t = jnp.tanh(GELU_C * g * (1.0 + GELU_A * g2))
                hg = 0.5 * g
                gel = hg + hg * t
                dgel = 0.5 + 0.5 * t + hg * (1.0 - t * t) * (GELU_C + 3.0 * GELU_A * GELU_C * g2)
                af = gel * u
                a = af.astype(bf16)
                dg = (da * u * dgel).astype(bf16)
                du = (da * gel).astype(bf16)
                y_acc[...] += _dot(a, wd_v[c])
                dhn_acc[...] += _dot_nt(dg, wg_v[c]) + _dot_nt(du, wu_v[c])
                ht = _upk(hnt[...])
                a_wg[c] = acc(a_wg[c], _dot(ht, dg))
                a_wu[c] = acc(a_wu[c], _dot(ht, du))
                a_wd[c] = acc(a_wd[c], _dot(af.T, gy_v[pl.ds(r0, TQ), :]))

            def ffn_pair(i, c):
                r_0 = ffn_a(2 * i)
                r_1 = ffn_a(2 * i + 1)
                ffn_b(2 * i, *r_0)
                ffn_b(2 * i + 1, *r_1)
                return c

            jax.lax.fori_loop(0, NFC // 2, ffn_pair, 0)

            rn = pl.multiple_of(jnp.minimum(qb + 1, NB - 1) * TQ, TQ)
            da_v[0] = _dot_nt(gy_v[pl.ds(rn, TQ), :], wd_v[0])

            h2_v[pl.ds(r0, TQ), :] = y_acc[...].astype(bf16)
            dh = gy_v[pl.ds(r0, TQ), :].astype(f32) + _layernorm_bwd(
                dhn_acc[...], hn_f[...], rstd_v[...])
            dh_v[pl.ds(r0, TQ), :] = dh
            dhb = dh.astype(bf16)
            dot_[...] = _dot_nt(wo_v[...], dhb)
            a_wo[...] = acc(a_wo[...], _dot(_upk(otb[...]), dhb))

            def head_terms(h):
                g, cg, ro, ws, off = _head_scalars(h)
                li = linv[h][0:1, :]
                dg_ = dot_[pl.ds(pl.multiple_of(cg, 8), 128), :]
                w = jnp.where(_row_mask(128, ro), dg_ * li, 0.0).astype(bf16)
                rs = pl.ds(pl.multiple_of(ws, 8), 24)
                m24 = _row_mask(24, off)
                do_l = jnp.where(m24, dot_[rs, :] * li, 0.0)
                delta = jnp.sum(do_l * ot[rs, :], axis=0, keepdims=True)
                return h, g, w, rs, m24, do_l, delta

            def ds_chunk(t, c):
                h, g, w, _, _, _, delta = t
                parts = []
                for s0 in range(0, CK, SUB):
                    r = c * CK + s0
                    parts.append(_dot(_upk(vnat[_prow(g, r // 2, SUB // 2), :]), w))
                dp = jnp.concatenate(parts, axis=0)
                p = _upk(p_refs[c][_pslot(h), :])
                return (p.astype(f32) * (dp - delta)).astype(bf16)

            ds0[...] = pltpu.bitcast(ds_chunk(head_terms(0), 0), u32)
            pltpu.make_async_copy(h2_v.at[pl.ds(r0, TQ), :], h2_hbm.at[pl.ds(r0, TQ), :],
                                  sem_h2.at[qb]).start()

            def bwd_iter(i, carry2):
                hs = [HPB * i + k for k in range(HPB)]
                terms = [head_terms(h) for h in hs]
                terms.append(head_terms(jnp.minimum(hs[-1] + 1, H - 1)))
                ds = _upk(ds0[...])
                dq = None
                for n in range(HPB * NCK):
                    k, c = divmod(n, NCK)
                    h, _, _, rs, m24, do_l, _ = terms[k]
                    if c == 0:
                        q_l = jnp.where(m24, qt[qb, rs, :], 0.0)
                    kn, cn = divmod(n + 1, NCK)
                    ds_next = ds_chunk(terms[kn], cn)
                    sl = pl.ds(c * CK, CK)
                    p = _upk(p_refs[c][_pslot(h, z), :])
                    dvt[rs, sl] += _dot_nt(do_l, p)
                    dkt[rs, sl] += _dot_nt(q_l, ds)
                    dqc = _dot(kt[rs, sl], ds)
                    dq = dqc if c == 0 else dq + dqc
                    if c == NCK - 1:
                        dqb[rs, :] = jnp.where(m24, dq * SCALE, dqb[rs, :])
                    ds = ds_next
                ds0[...] = pltpu.bitcast(ds, u32)
                return carry2

            jax.lax.fori_loop(0, H // HPB, bwd_iter, 0)
            return carry

        jax.lax.fori_loop(0, NB, qblock, 0)
        save_dq(NB - 1)

    main()

    w_copies = [pltpu.make_async_copy(wo_v, dwo_hbm, sem_w.at[0])]
    for c in range(NFC):
        cs = pl.ds(c * FC, FC)
        w_copies += [pltpu.make_async_copy(wg_v.at[c], dwg_hbm.at[:, cs], sem_w.at[1 + 3 * c]),
                     pltpu.make_async_copy(wu_v.at[c], dwu_hbm.at[:, cs], sem_w.at[2 + 3 * c]),
                     pltpu.make_async_copy(wd_v.at[c], dwd_hbm.at[cs, :], sem_w.at[3 + 3 * c])]

    RW = D // NB

    def blk_a(b, carry):
        cs = pl.ds(pl.multiple_of(b * TQ, TQ), TQ)
        rd = pl.ds(pl.multiple_of(b * (D // 2), 8), D // 2)
        dq_p = dqt[rd, :]
        dk_b = (dkt[:, cs] * LN2).astype(bf16)
        dv_b = dvt[:, cs].astype(bf16)
        qt[b] = (_dot(wqkv_v[:, 0:D], _upk(dq_p)) + _dot(wqkv_v[:, D:2 * D], dk_b)
                 + _dot(wqkv_v[:, 2 * D:3 * D], dv_b))
        p_refs[0][rd, :] = pltpu.bitcast(dk_b, u32)
        p_refs[1][rd, :] = pltpu.bitcast(dv_b, u32)
        ra = pl.ds(pl.multiple_of(b * RW, 16), RW)
        rb = pl.ds(pl.multiple_of(b * (FC // NB), 16), FC // NB)
        wo_v[ra, :] = a_wo[ra, :].astype(bf16)
        for c in range(NFC):
            wg_v[c, ra, :] = a_wg[c, ra, :].astype(bf16)
            wu_v[c, ra, :] = a_wu[c, ra, :].astype(bf16)
            wd_v[c, rb, :] = a_wd[c, rb, :].astype(bf16)
        return carry

    jax.lax.fori_loop(0, NB, blk_a, 0)
    for cp in w_copies:
        cp.start()

    def blk_b(b, carry):
        cs = pl.ds(pl.multiple_of(b * TQ, TQ), TQ)
        ra = pl.ds(pl.multiple_of(b * RW, 16), RW)
        xr = pl.ds(pl.multiple_of(b * (RW // 2), 8), RW // 2)
        for j, src in enumerate((dqt, p_refs[0], p_refs[1])):
            for n in range(D // WC):
                acc_w = None
                for t in range(NB):
                    r = t * (D // 2) + n * (WC // 2)
                    part = _dot_nt(_upk(xnt[xr, t * TQ:(t + 1) * TQ]), _upk(src[r:r + WC // 2, :]))
                    acc_w = part if acc_w is None else acc_w + part
                wqkv_v[ra, j * D + n * WC:j * D + (n + 1) * WC] = acc_w.astype(bf16)
        xn, rstd = _layernorm(x_v[cs, :].astype(f32))
        dx = dh_v[cs, :] + _layernorm_bwd(qt[b].T, xn, rstd)
        gy_v[cs, :] = dx.astype(bf16)
        pltpu.make_async_copy(gy_v.at[cs, :], dx_hbm.at[cs, :], sem_dx.at[b]).start()
        pltpu.make_async_copy(wqkv_v.at[ra, :], dwqkv_hbm.at[ra, :], sem_wq.at[b]).start()
        return carry

    jax.lax.fori_loop(0, NB, blk_b, 0)
    for b in range(NB):
        ra = pl.ds(b * RW, RW)
        pltpu.make_async_copy(wqkv_v.at[ra, :], dwqkv_hbm.at[ra, :], sem_wq.at[b]).wait()

    for b in range(NB):
        rs = pl.ds(b * TQ, TQ)
        pltpu.make_async_copy(h2_v.at[rs, :], h2_hbm.at[rs, :], sem_h2.at[b]).wait()
        pltpu.make_async_copy(gy_v.at[rs, :], dx_hbm.at[rs, :], sem_dx.at[b]).wait()
    for cp in w_copies:
        cp.wait()


@jax.jit
def pallas_sequential_preLN__softmax_full_mha__glu_gated_geglu__prompt_kernel(
    A_x: jax.Array,
    A_wqkv: jax.Array,
    A_wo: jax.Array,
    B_x: jax.Array,
    B_w_gate: jax.Array,
    B_w_up: jax.Array,
    B_w_down: jax.Array,
    grad_out: jax.Array,
):
    del B_x
    any_spec = pl.BlockSpec(memory_space=pl.ANY)
    out_shape = (
        jax.ShapeDtypeStruct((S, D), bf16),
        jax.ShapeDtypeStruct((S, D), bf16),
        jax.ShapeDtypeStruct((D, 3 * D), bf16),
        jax.ShapeDtypeStruct((D, D), bf16),
        jax.ShapeDtypeStruct((D, DF), bf16),
        jax.ShapeDtypeStruct((D, DF), bf16),
        jax.ShapeDtypeStruct((DF, D), bf16),
    )
    scratch = [
        pltpu.VMEM((S, D), bf16),
        pltpu.VMEM((S, D), bf16),
        pltpu.VMEM((D, 3 * D), bf16),
        pltpu.VMEM((D, D), bf16),
        pltpu.VMEM((NFC, D, FC), bf16),
        pltpu.VMEM((NFC, D, FC), bf16),
        pltpu.VMEM((NFC, FC, D), bf16),
        pltpu.VMEM((S, D), bf16),
        pltpu.VMEM((NB, D, TQ), f32),
        pltpu.VMEM((NG * S // 2, 128), u32),
        pltpu.VMEM((NG * S // 2, 128), u32),
        pltpu.VMEM((D, S), f32),
        pltpu.VMEM((D, S), f32),
        pltpu.VMEM((D // 2, S), u32),
        pltpu.VMEM((D, S), f32),
        pltpu.VMEM((D, S), f32),
        pltpu.VMEM((NB * D // 2, TQ), u32),
        pltpu.VMEM((S, D), f32),
        pltpu.VMEM((NFC, D, FC), f32),
        pltpu.VMEM((NFC, D, FC), f32),
        pltpu.VMEM((NFC, FC, D), f32),
        pltpu.VMEM((D, D), f32),
        [pltpu.VMEM((H * S // 2 // NP, TQ), u32)] * NP,
        [pltpu.VMEM((S // NS, TQ), f32)] * NS,
        [pltpu.VMEM((S // NS, TQ), f32)] * NS,
        pltpu.VMEM((8, TQ), f32),
        pltpu.VMEM((D, TQ), f32),
        pltpu.VMEM((D, TQ), f32),
        pltpu.VMEM((D, TQ), f32),
        pltpu.VMEM((H, 8, TQ), f32),
        pltpu.VMEM((TQ, D), f32),
        pltpu.VMEM((TQ // 2, D), u32),
        pltpu.VMEM((D // 2, TQ), u32),
        pltpu.VMEM((D // 2, TQ), u32),
        pltpu.VMEM((TQ, D), f32),
        pltpu.VMEM((TQ, D), f32),
        pltpu.VMEM((TQ, 1), f32),
        pltpu.VMEM((NFC, TQ, FC), f32),
        pltpu.VMEM((CK // 2, TQ), u32),
        pltpu.SemaphoreType.DMA((NB,)),
        pltpu.SemaphoreType.DMA((3,)),
        pltpu.SemaphoreType.DMA((2 + 3 * NFC,)),
        pltpu.SemaphoreType.DMA((NB,)),
        pltpu.SemaphoreType.DMA((NB,)),
        pltpu.SemaphoreType.DMA((1 + 3 * NFC,)),
        pltpu.SemaphoreType.DMA((NB,)),
    ]
    outs = pl.pallas_call(
        _kernel,
        out_shape=out_shape,
        in_specs=[any_spec] * 7,
        out_specs=[any_spec] * 7,
        scratch_shapes=scratch,
        compiler_params=pltpu.CompilerParams(vmem_limit_bytes=124 * 1024 * 1024),
    )(A_x.reshape(S, D), A_wqkv, A_wo, B_w_gate, B_w_up, B_w_down, grad_out.reshape(S, D))
    h2, dx, dwqkv, dwo, dwg, dwu, dwd = outs
    return (h2.reshape(1, S, D), dx.reshape(1, S, D), dwqkv, dwo, dwg, dwu, dwd)
```

```python
import math

import jax
import jax.numpy as jnp
import jax.experimental.pallas as pl
import jax.experimental.pallas.tpu as pltpu

f32 = jnp.float32
bf16 = jnp.bfloat16
u32 = jnp.uint32

S = 2048
D = 640
H = 32
DH = 20
DF = 1536
TQ = 256
NB = S // TQ
FC = 256
NFC = DF // FC
HG = 4
NG = H // HG
CK = 256
SUB = 128
NCK = S // CK
WC = 128
EPS = 1e-5
SCALE = DH ** -0.5
QSCALE = SCALE * math.log2(math.e)
LN2 = math.log(2.0)
GELU_C = math.sqrt(2.0 / math.pi)
GELU_A = 0.044715

NN = (((1,), (0,)), ((), ()))
NT = (((1,), (1,)), ((), ()))
HPF = 8
HPB = 8
NS = 2
ZB = 5
MS = 320
LAG = 1


def _dot(a, b):
    return jax.lax.dot_general(a, b, NN, preferred_element_type=f32)


def _dot_nt(a, b):
    return jax.lax.dot_general(a, b, NT, preferred_element_type=f32)


def _pk(x):
    return pltpu.bitcast(x.astype(bf16), u32)


def _upk(x):
    return pltpu.bitcast(x, bf16)


def _prow(i, start, size):
    return pl.ds(pl.multiple_of(i * (S // 2) + start, 8), size)


def _pslot(h0, k, z=0):
    return pl.ds(pl.multiple_of(z + h0 * (CK // 2) + k * (CK // 2), 8), CK // 2)


def _layernorm(x):
    mu = jnp.mean(x, axis=-1, keepdims=True)
    xc = x - mu
    var = jnp.mean(xc * xc, axis=-1, keepdims=True)
    rstd = jax.lax.rsqrt(var + EPS)
    return xc * rstd, rstd


def _layernorm_bwd(dy, y, rstd):
    m1 = jnp.mean(dy, axis=-1, keepdims=True)
    m2 = jnp.mean(dy * y, axis=-1, keepdims=True)
    return rstd * (dy - m1 - y * m2)


def _head_window(h0, k):
    ws = DH * h0 + (DH * k // 8) * 8
    return pl.ds(pl.multiple_of(ws, 8), 24), DH * k % 8


def _group_weights(win, k):
    lo = (DH * (k % HG) // 8) * 8
    parts = [jnp.zeros((lo, TQ), f32)] if lo else []
    parts += [win, jnp.zeros((128 - 24 - lo, TQ), f32)]
    return jnp.concatenate(parts, axis=0).astype(bf16)


def _row_mask(nrows, lo):
    r = jax.lax.broadcasted_iota(jnp.int32, (nrows, TQ), 0)
    return jnp.logical_and(r >= lo, r < lo + DH)


def _kernel(x_hbm, wqkv_hbm, wo_hbm, wg_hbm, wu_hbm, wd_hbm, gy_hbm,
            h2_hbm, dx_hbm, dwqkv_hbm, dwo_hbm, dwg_hbm, dwu_hbm, dwd_hbm,
            x_v, gy_v, wqkv_v, wo_v, wg_v, wu_v, wd_v, h2_v,
            qt, knat, vnat, kt, vt, xnt, dkt, dvt, dqt, dh_v,
            a_wg, a_wu, a_wd, a_wo,
            p_refs, s_a, s_b, m_v, ot, dot_, dqb, linv, hn_f, hn_b, hnt,
            otb, y_acc, dhn_acc, rstd_v, da_v, ds0,
            sem_x, sem_qkv, sem_in, sem_h2, sem_dx, sem_w, sem_wq):

    def x_copy(b):
        rs = pl.ds(pl.multiple_of(b * TQ, TQ), TQ)
        return pltpu.make_async_copy(x_hbm.at[rs, :], x_v.at[rs, :], sem_x.at[b])

    qkv_copies = [pltpu.make_async_copy(wqkv_hbm.at[:, pl.ds(t * D, D)],
                                        wqkv_v.at[:, pl.ds(t * D, D)], sem_qkv.at[t])
                  for t in range(3)]
    in_copies = [pltpu.make_async_copy(wo_hbm, wo_v, sem_in.at[0]),
                 pltpu.make_async_copy(gy_hbm, gy_v, sem_in.at[1])]
    for c in range(NFC):
        cs = pl.ds(c * FC, FC)
        in_copies.append(pltpu.make_async_copy(wg_hbm.at[:, cs], wg_v.at[c], sem_in.at[2 + 3 * c]))
        in_copies.append(pltpu.make_async_copy(wu_hbm.at[:, cs], wu_v.at[c], sem_in.at[3 + 3 * c]))
        in_copies.append(pltpu.make_async_copy(wd_hbm.at[cs, :], wd_v.at[c], sem_in.at[4 + 3 * c]))

    x_copy(0).start()
    qkv_copies[1].start()

    def zero_blk(b, carry):
        cs = pl.ds(pl.multiple_of(b * TQ, TQ), TQ)
        dkt[:, cs] = jnp.zeros((D, TQ), f32)
        dvt[:, cs] = jnp.zeros((D, TQ), f32)
        return carry

    jax.lax.fori_loop(0, ZB, zero_blk, 0)
    qkv_copies[2].start()
    x_copy(1).start()
    jax.lax.fori_loop(ZB, NB, zero_blk, 0)

    def ln_block(b):
        r0 = pl.multiple_of(b * TQ, TQ)
        xn, _ = _layernorm(x_v[pl.ds(r0, TQ), :].astype(f32))
        xnt[:, pl.ds(r0, TQ)] = _pk(xn.T)
        return _pk(xn)

    def proj_block(b, first):
        r0 = pl.multiple_of(b * TQ, TQ)
        r2 = pl.multiple_of(b * (TQ // 2), TQ // 2)
        xb = _upk(hn_b[...])

        def finish(y, nat, tr):
            y_t = y.astype(bf16).astype(f32).T
            tr[:, pl.ds(r0, TQ)] = y_t
            y_p = jnp.concatenate([y_t, jnp.zeros((48, TQ), f32)], axis=0)
            for g in range(NG):
                c0 = HG * DH * g
                nat[_prow(g, r2, TQ // 2), :] = _pk(y_p[c0:c0 + 128].T)

        if first:
            qkv_copies[1].wait()
            qkv_copies[0].start()
        k = _dot(xb, wqkv_v[:, D:2 * D])
        if first:
            qkv_copies[2].wait()
            x_copy(1).wait()
            v = _dot(xb, wqkv_v[:, 2 * D:3 * D])
            finish(k, knat, kt)
            for bb in range(2, NB):
                x_copy(bb).start()
            qkv_copies[0].wait()
            q = _dot(xb, wqkv_v[:, 0:D]) * QSCALE
            xb_next = ln_block(1)
            finish(v, vnat, vt)
        else:
            xb_next = ln_block(jnp.minimum(b + 1, NB - 1))
            finish(k, knat, kt)
            finish(_dot(xb, wqkv_v[:, 2 * D:3 * D]), vnat, vt)
            q = _dot(xb, wqkv_v[:, 0:D]) * QSCALE
        qt[b] = q.T
        hn_b[...] = xb_next

    def phase0():
        x_copy(0).wait()
        hn_b[...] = ln_block(0)
        proj_block(0, True)
        for cp in in_copies:
            cp.start()

        def blk(b, carry):
            @pl.when(b + 1 < NB)
            def _():
                x_copy(b + 1).wait()

            proj_block(b, False)
            return carry

        jax.lax.fori_loop(1, NB, blk, 0)

    phase0()

    for cp in in_copies:
        cp.wait()

    def main():
        ot[...] = jnp.zeros_like(ot)
        dqb[...] = jnp.zeros_like(dqb)
        sbuf = (s_a, s_b)
        HC = NCK // NS

        def save_dq(b):
            dqt[pl.ds(pl.multiple_of(b * (D // 2), 8), D // 2), :] = _pk(dqb[...])

        def score_weights(qn, h0, k):
            rs, off = _head_window(h0, k)
            win = jnp.where(_row_mask(24, off), qt[qn, rs, :], 0.0)
            return h0 // HG + k // HG, _group_weights(win, k)

        def score_chunk(g, w, c, dst, m):
            for s0 in range(0, CK, SUB):
                r = c * CK + s0
                s = _dot(_upk(knat[_prow(g, r // 2, SUB // 2), :]), w)
                dst[c // HC][pl.ds((c % HC) * CK + s0, SUB), :] = s
                mc = jnp.max(s.reshape(SUB // 8, 8, TQ), axis=0)
                m = mc if m is None else jnp.maximum(m, mc)
            return m

        g0, w0 = score_weights(0, 0, 0)
        m0 = None
        for c in range(NCK):
            m0 = score_chunk(g0, w0, c, sbuf[0], m0)
        m_v[...] = jnp.broadcast_to(jnp.max(m0, axis=0, keepdims=True), (8, TQ))
        da_v[0] = _dot_nt(gy_v[0:TQ, :], wd_v[0])

        def qblock(qb, carry):
            r0 = pl.multiple_of(qb * TQ, TQ)
            z = jax.lax.shift_right_logical(qb, 20) * 8
            later = qb > 0

            def acc(old, new):
                return jnp.where(later, old, 0.0) + new

            def fwd_iter(i, carry2):
                h0 = HPF * i
                wrap = jax.lax.shift_right_logical(h0 + HPF, 5)
                nxt = [(qb, h0, k + 1) for k in range(HPF - 1)]
                nxt.append((jnp.minimum(qb + wrap, NB - 1), jnp.bitwise_and(h0 + HPF, H - 1), 0))
                mrow = [m_v[0:1, :]]
                rows = jax.lax.broadcasted_iota(jnp.int32, (24, CK), 0)
                n_steps = HPF * NCK
                m = o = gw = None
                for n in range(n_steps + LAG):
                    if n < n_steps:
                        k, c = divmod(n, NCK)
                        if c == 0:
                            gw = score_weights(*nxt[k])
                            m = None
                        m = score_chunk(gw[0], gw[1], c, sbuf[(k + 1) % 2], m)
                        if c == NCK - 1:
                            mrow.append(jnp.max(m, axis=0, keepdims=True))
                    if n >= LAG:
                        k, c = divmod(n - LAG, NCK)
                        rs, off = _head_window(h0, k)
                        one = 23 if off == 0 else 0
                        src = sbuf[k % 2][c // HC]
                        sv = src[pl.ds(pl.multiple_of(z + (c % HC) * CK, 8), CK), :]
                        p = jnp.exp2(sv - mrow[k]).astype(bf16)
                        p_refs[c][_pslot(h0, k), :] = pltpu.bitcast(p, u32)
                        vl = jnp.where(rows == one, 1.0, vt[rs, pl.ds(c * CK, CK)])
                        oc = _dot(vl, p)
                        o = oc if c == 0 else o + oc
                        if c == NCK - 1:
                            li = 1.0 / o[one:one + 1]
                            linv[h0 + k] = jnp.broadcast_to(li, (8, TQ))
                            ot[rs, :] = jnp.where(_row_mask(24, off), o * li, ot[rs, :])
                m_v[...] = jnp.broadcast_to(mrow[-1], (8, TQ))
                return carry2

            jax.lax.fori_loop(0, H // HPF, fwd_iter, 0)

            gyb = gy_v[pl.ds(r0, TQ), :]
            da_v[1] = _dot_nt(gyb, wd_v[1])
            save_dq(jnp.maximum(qb - 1, 0))
            o_t = ot[...]
            otb[...] = _pk(o_t)
            attn = _dot(o_t.T.astype(bf16), wo_v[...])
            dhn_acc[...] = jnp.zeros_like(dhn_acc)
            hres = x_v[pl.ds(r0, TQ), :].astype(f32) + attn
            y_acc[...] = hres
            hn, rstd = _layernorm(hres)
            hn_f[...] = hn
            rstd_v[...] = rstd
            hn_b[...] = _pk(hn)
            hnt[...] = _pk(hn.T)
            for c in range(2, NFC):
                da_v[c] = _dot_nt(gyb, wd_v[c])

            def ffn_a(c):
                hb = _upk(hn_b[...])
                g = _dot(hb, wg_v[c])
                u = _dot(hb, wu_v[c])
                return g, u

            def ffn_b(c, g, u):
                da = da_v[c]
                g2 = g * g
                t = jnp.tanh(GELU_C * g * (1.0 + GELU_A * g2))
                hg = 0.5 * g
                gel = hg + hg * t
                dgel = 0.5 + 0.5 * t + hg * (1.0 - t * t) * (GELU_C + 3.0 * GELU_A * GELU_C * g2)
                af = gel * u
                a = af.astype(bf16)
                dg = (da * u * dgel).astype(bf16)
                du = (da * gel).astype(bf16)
                y_acc[...] += _dot(a, wd_v[c])
                dhn_acc[...] += _dot_nt(dg, wg_v[c]) + _dot_nt(du, wu_v[c])
                ht = _upk(hnt[...])
                a_wg[c] = acc(a_wg[c], _dot(ht, dg))
                a_wu[c] = acc(a_wu[c], _dot(ht, du))
                a_wd[c] = acc(a_wd[c], _dot(af.T, gy_v[pl.ds(r0, TQ), :]))

            def ffn_pair(i, c):
                r_0 = ffn_a(2 * i)
                r_1 = ffn_a(2 * i + 1)
                ffn_b(2 * i, *r_0)
                ffn_b(2 * i + 1, *r_1)
                return c

            jax.lax.fori_loop(0, NFC // 2, ffn_pair, 0)

            rn = pl.multiple_of(jnp.minimum(qb + 1, NB - 1) * TQ, TQ)
            da_v[0] = _dot_nt(gy_v[pl.ds(rn, TQ), :], wd_v[0])

            h2_v[pl.ds(r0, TQ), :] = y_acc[...].astype(bf16)
            dh = gy_v[pl.ds(r0, TQ), :].astype(f32) + _layernorm_bwd(
                dhn_acc[...], hn_f[...], rstd_v[...])
            dh_v[pl.ds(r0, TQ), :] = dh
            dhb = dh.astype(bf16)
            dot_[...] = _dot_nt(wo_v[...], dhb)
            a_wo[...] = acc(a_wo[...], _dot(_upk(otb[...]), dhb))

            def head_terms(h0, k):
                rs, off = _head_window(h0, k)
                m24 = _row_mask(24, off)
                do_l = jnp.where(m24, dot_[rs, :] * linv[h0 + k][0:1, :], 0.0)
                delta = jnp.sum(do_l * ot[rs, :], axis=0, keepdims=True)
                return h0, k, _group_weights(do_l, k), rs, m24, do_l, delta

            def ds_chunk(t, c):
                h0, k, w, _, _, _, delta = t
                parts = []
                for s0 in range(0, CK, SUB):
                    r = c * CK + s0
                    parts.append(
                        _dot(_upk(vnat[_prow(h0 // HG + k // HG, r // 2, SUB // 2), :]), w))
                dp = jnp.concatenate(parts, axis=0)
                p = _upk(p_refs[c][_pslot(h0, k), :])
                return (p.astype(f32) * (dp - delta)).astype(bf16)

            ds0[...] = pltpu.bitcast(ds_chunk(head_terms(0, 0), 0), u32)
            pltpu.make_async_copy(h2_v.at[pl.ds(r0, TQ), :], h2_hbm.at[pl.ds(r0, TQ), :],
                                  sem_h2.at[qb]).start()

            def bwd_iter(i, carry2):
                h0 = HPB * i
                terms = [head_terms(h0, k) for k in range(HPB)]
                terms.append(head_terms(jnp.minimum(h0 + HPB, H - HPB), 0))
                ds = _upk(ds0[...])
                dq = None
                for n in range(HPB * NCK):
                    k, c = divmod(n, NCK)
                    _, _, _, rs, m24, do_l, _ = terms[k]
                    if c == 0:
                        q_l = jnp.where(m24, qt[qb, rs, :], 0.0)
                    kn, cn = divmod(n + 1, NCK)
                    ds_next = ds_chunk(terms[kn], cn)
                    sl = pl.ds(c * CK, CK)
                    p = _upk(p_refs[c][_pslot(h0, k, z), :])
                    dvt[rs, sl] += _dot_nt(do_l, p)
                    dkt[rs, sl] += _dot_nt(q_l, ds)
                    dqc = _dot(kt[rs, sl], ds)
                    dq = dqc if c == 0 else dq + dqc
                    if c == NCK - 1:
                        dqb[rs, :] = jnp.where(m24, dq * SCALE, dqb[rs, :])
                    ds = ds_next
                ds0[...] = pltpu.bitcast(ds, u32)
                return carry2

            jax.lax.fori_loop(0, H // HPB, bwd_iter, 0)
            return carry

        jax.lax.fori_loop(0, NB, qblock, 0)
        save_dq(NB - 1)

    main()

    w_copies = [pltpu.make_async_copy(wo_v, dwo_hbm, sem_w.at[0])]
    for c in range(NFC):
        cs = pl.ds(c * FC, FC)
        w_copies += [pltpu.make_async_copy(wg_v.at[c], dwg_hbm.at[:, cs], sem_w.at[1 + 3 * c]),
                     pltpu.make_async_copy(wu_v.at[c], dwu_hbm.at[:, cs], sem_w.at[2 + 3 * c]),
                     pltpu.make_async_copy(wd_v.at[c], dwd_hbm.at[cs, :], sem_w.at[3 + 3 * c])]

    RW = D // NB

    def blk_a(b, carry):
        cs = pl.ds(pl.multiple_of(b * TQ, TQ), TQ)
        rd = pl.ds(pl.multiple_of(b * (D // 2), 8), D // 2)
        dq_p = dqt[rd, :]
        dk_b = (dkt[:, cs] * LN2).astype(bf16)
        dv_b = dvt[:, cs].astype(bf16)
        for m0 in range(0, D, MS):
            ms = slice(m0, m0 + MS)
            qt[b, ms, :] = (_dot(wqkv_v[ms, 0:D], _upk(dq_p)) + _dot(wqkv_v[ms, D:2 * D], dk_b)
                            + _dot(wqkv_v[ms, 2 * D:3 * D], dv_b))
        p_refs[0][rd, :] = pltpu.bitcast(dk_b, u32)
        p_refs[1][rd, :] = pltpu.bitcast(dv_b, u32)
        ra = pl.ds(pl.multiple_of(b * RW, 16), RW)
        rb = pl.ds(pl.multiple_of(b * (FC // NB), 16), FC // NB)
        wo_v[ra, :] = a_wo[ra, :].astype(bf16)
        for c in range(NFC):
            wg_v[c, ra, :] = a_wg[c, ra, :].astype(bf16)
            wu_v[c, ra, :] = a_wu[c, ra, :].astype(bf16)
            wd_v[c, rb, :] = a_wd[c, rb, :].astype(bf16)
        return carry

    jax.lax.fori_loop(0, NB, blk_a, 0)
    for cp in w_copies:
        cp.start()

    def blk_b(b, carry):
        cs = pl.ds(pl.multiple_of(b * TQ, TQ), TQ)
        ra = pl.ds(pl.multiple_of(b * RW, 16), RW)
        xr = pl.ds(pl.multiple_of(b * (RW // 2), 8), RW // 2)
        xn, rstd = _layernorm(x_v[cs, :].astype(f32))
        dx = dh_v[cs, :] + _layernorm_bwd(qt[b].T, xn, rstd)
        gy_v[cs, :] = dx.astype(bf16)
        for j, src in enumerate((dqt, p_refs[0], p_refs[1])):
            for n in range(D // WC):
                acc_w = None
                for t in range(NB):
                    r = t * (D // 2) + n * (WC // 2)
                    part = _dot_nt(_upk(xnt[xr, t * TQ:(t + 1) * TQ]), _upk(src[r:r + WC // 2, :]))
                    acc_w = part if acc_w is None else acc_w + part
                wqkv_v[ra, j * D + n * WC:j * D + (n + 1) * WC] = acc_w.astype(bf16)
        pltpu.make_async_copy(gy_v.at[cs, :], dx_hbm.at[cs, :], sem_dx.at[b]).start()
        pltpu.make_async_copy(wqkv_v.at[ra, :], dwqkv_hbm.at[ra, :], sem_wq.at[b]).start()
        return carry

    jax.lax.fori_loop(0, NB, blk_b, 0)

    for b in range(NB):
        rs = pl.ds(b * TQ, TQ)
        pltpu.make_async_copy(h2_v.at[rs, :], h2_hbm.at[rs, :], sem_h2.at[b]).wait()
    for cp in w_copies:
        cp.wait()
    for b in range(NB):
        rs = pl.ds(b * TQ, TQ)
        ra = pl.ds(b * RW, RW)
        pltpu.make_async_copy(gy_v.at[rs, :], dx_hbm.at[rs, :], sem_dx.at[b]).wait()
        pltpu.make_async_copy(wqkv_v.at[ra, :], dwqkv_hbm.at[ra, :], sem_wq.at[b]).wait()


@jax.jit
def pallas_sequential_preLN__softmax_full_mha__glu_gated_geglu__prompt_kernel(
    A_x: jax.Array,
    A_wqkv: jax.Array,
    A_wo: jax.Array,
    B_x: jax.Array,
    B_w_gate: jax.Array,
    B_w_up: jax.Array,
    B_w_down: jax.Array,
    grad_out: jax.Array,
):
    del B_x
    any_spec = pl.BlockSpec(memory_space=pl.ANY)
    out_shape = (
        jax.ShapeDtypeStruct((S, D), bf16),
        jax.ShapeDtypeStruct((S, D), bf16),
        jax.ShapeDtypeStruct((D, 3 * D), bf16),
        jax.ShapeDtypeStruct((D, D), bf16),
        jax.ShapeDtypeStruct((D, DF), bf16),
        jax.ShapeDtypeStruct((D, DF), bf16),
        jax.ShapeDtypeStruct((DF, D), bf16),
    )
    scratch = [
        pltpu.VMEM((S, D), bf16),
        pltpu.VMEM((S, D), bf16),
        pltpu.VMEM((D, 3 * D), bf16),
        pltpu.VMEM((D, D), bf16),
        pltpu.VMEM((NFC, D, FC), bf16),
        pltpu.VMEM((NFC, D, FC), bf16),
        pltpu.VMEM((NFC, FC, D), bf16),
        pltpu.VMEM((S, D), bf16),
        pltpu.VMEM((NB, D, TQ), f32),
        pltpu.VMEM((NG * S // 2, 128), u32),
        pltpu.VMEM((NG * S // 2, 128), u32),
        pltpu.VMEM((D, S), f32),
        pltpu.VMEM((D, S), f32),
        pltpu.VMEM((D // 2, S), u32),
        pltpu.VMEM((D, S), f32),
        pltpu.VMEM((D, S), f32),
        pltpu.VMEM((NB * D // 2, TQ), u32),
        pltpu.VMEM((S, D), f32),
        pltpu.VMEM((NFC, D, FC), f32),
        pltpu.VMEM((NFC, D, FC), f32),
        pltpu.VMEM((NFC, FC, D), f32),
        pltpu.VMEM((D, D), f32),
        [pltpu.VMEM((H * CK // 2, TQ), u32)] * NCK,
        [pltpu.VMEM((S // NS, TQ), f32)] * NS,
        [pltpu.VMEM((S // NS, TQ), f32)] * NS,
        pltpu.VMEM((8, TQ), f32),
        pltpu.VMEM((D, TQ), f32),
        pltpu.VMEM((D, TQ), f32),
        pltpu.VMEM((D, TQ), f32),
        pltpu.VMEM((H, 8, TQ), f32),
        pltpu.VMEM((TQ, D), f32),
        pltpu.VMEM((TQ // 2, D), u32),
        pltpu.VMEM((D // 2, TQ), u32),
        pltpu.VMEM((D // 2, TQ), u32),
        pltpu.VMEM((TQ, D), f32),
        pltpu.VMEM((TQ, D), f32),
        pltpu.VMEM((TQ, 1), f32),
        pltpu.VMEM((NFC, TQ, FC), f32),
        pltpu.VMEM((CK // 2, TQ), u32),
        pltpu.SemaphoreType.DMA((NB,)),
        pltpu.SemaphoreType.DMA((3,)),
        pltpu.SemaphoreType.DMA((2 + 3 * NFC,)),
        pltpu.SemaphoreType.DMA((NB,)),
        pltpu.SemaphoreType.DMA((NB,)),
        pltpu.SemaphoreType.DMA((1 + 3 * NFC,)),
        pltpu.SemaphoreType.DMA((NB,)),
    ]
    outs = pl.pallas_call(
        _kernel,
        out_shape=out_shape,
        in_specs=[any_spec] * 7,
        out_specs=[any_spec] * 7,
        scratch_shapes=scratch,
        compiler_params=pltpu.CompilerParams(vmem_limit_bytes=124 * 1024 * 1024),
    )(A_x.reshape(S, D), A_wqkv, A_wo, B_w_gate, B_w_up, B_w_down, grad_out.reshape(S, D))
    h2, dx, dwqkv, dwo, dwg, dwu, dwd = outs
    return (h2.reshape(1, S, D), dx.reshape(1, S, D), dwqkv, dwo, dwg, dwu, dwd)
```

```python
import math

import jax
import jax.numpy as jnp
import jax.experimental.pallas as pl
import jax.experimental.pallas.tpu as pltpu

f32 = jnp.float32
bf16 = jnp.bfloat16
u32 = jnp.uint32

S = 2048
D = 640
H = 32
DH = 20
DF = 1536
TQ = 256
NB = S // TQ
FC = 256
NFC = DF // FC
HG = 4
NG = H // HG
CK = 256
SUB = 128
NCK = S // CK
WC = 128
EPS = 1e-5
SCALE = DH ** -0.5
QSCALE = SCALE * math.log2(math.e)
LN2 = math.log(2.0)
GELU_C = math.sqrt(2.0 / math.pi)
GELU_A = 0.044715

NN = (((1,), (0,)), ((), ()))
NT = (((1,), (1,)), ((), ()))
HPF = 8
HPB = 8
NS = 2
ZB = 5
MS = 320
LAG = 1


def _dot(a, b):
    return jax.lax.dot_general(a, b, NN, preferred_element_type=f32)


def _dot_nt(a, b):
    return jax.lax.dot_general(a, b, NT, preferred_element_type=f32)


def _pk(x):
    return pltpu.bitcast(x.astype(bf16), u32)


def _upk(x):
    return pltpu.bitcast(x, bf16)


def _prow(i, start, size):
    return pl.ds(pl.multiple_of(i * (S // 2) + start, 8), size)


def _pslot(h0, k, z=0):
    return pl.ds(pl.multiple_of(z + h0 * (CK // 2) + k * (CK // 2), 8), CK // 2)


def _layernorm(x):
    mu = jnp.mean(x, axis=-1, keepdims=True)
    xc = x - mu
    var = jnp.mean(xc * xc, axis=-1, keepdims=True)
    rstd = jax.lax.rsqrt(var + EPS)
    return xc * rstd, rstd


def _layernorm_bwd(dy, y, rstd):
    m1 = jnp.mean(dy, axis=-1, keepdims=True)
    m2 = jnp.mean(dy * y, axis=-1, keepdims=True)
    return rstd * (dy - m1 - y * m2)


def _head_window(h0, k):
    ws = DH * h0 + (DH * k // 8) * 8
    return pl.ds(pl.multiple_of(ws, 8), 24), DH * k % 8


def _group(h0, k):
    g0 = h0 // HG if isinstance(h0, int) else jax.lax.shift_right_logical(h0, 2)
    return g0 + k // HG


def _group_weights(win, k):
    lo = (DH * (k % HG) // 8) * 8
    parts = [jnp.zeros((lo, TQ), f32)] if lo else []
    parts += [win, jnp.zeros((128 - 24 - lo, TQ), f32)]
    return jnp.concatenate(parts, axis=0).astype(bf16)


def _row_mask(nrows, lo):
    r = jax.lax.broadcasted_iota(jnp.int32, (nrows, TQ), 0)
    return jnp.logical_and(r >= lo, r < lo + DH)


def _kernel(x_hbm, wqkv_hbm, wo_hbm, wg_hbm, wu_hbm, wd_hbm, gy_hbm,
            h2_hbm, dx_hbm, dwqkv_hbm, dwo_hbm, dwg_hbm, dwu_hbm, dwd_hbm,
            x_v, gy_v, wqkv_v, wo_v, wg_v, wu_v, wd_v, h2_v,
            qt, knat, vnat, kt, vt, xnt, dkt, dvt, dqt, dh_v,
            a_wg, a_wu, a_wd, a_wo,
            p_refs, s_a, s_b, m_v, ot, dot_, dqb, linv, hn_f, hn_b, hnt,
            otb, y_acc, dhn_acc, rstd_v, da_v, ds0,
            sem_x, sem_qkv, sem_in, sem_h2, sem_dx, sem_w, sem_wq):

    def x_copy(b):
        rs = pl.ds(pl.multiple_of(b * TQ, TQ), TQ)
        return pltpu.make_async_copy(x_hbm.at[rs, :], x_v.at[rs, :], sem_x.at[b])

    qkv_copies = [pltpu.make_async_copy(wqkv_hbm.at[:, pl.ds(t * D, D)],
                                        wqkv_v.at[:, pl.ds(t * D, D)], sem_qkv.at[t])
                  for t in range(3)]
    in_copies = [pltpu.make_async_copy(wo_hbm, wo_v, sem_in.at[0]),
                 pltpu.make_async_copy(gy_hbm, gy_v, sem_in.at[1])]
    for c in range(NFC):
        cs = pl.ds(c * FC, FC)
        in_copies.append(pltpu.make_async_copy(wg_hbm.at[:, cs], wg_v.at[c], sem_in.at[2 + 3 * c]))
        in_copies.append(pltpu.make_async_copy(wu_hbm.at[:, cs], wu_v.at[c], sem_in.at[3 + 3 * c]))
        in_copies.append(pltpu.make_async_copy(wd_hbm.at[cs, :], wd_v.at[c], sem_in.at[4 + 3 * c]))

    x_copy(0).start()
    qkv_copies[1].start()

    def zero_blk(b, carry):
        cs = pl.ds(pl.multiple_of(b * TQ, TQ), TQ)
        dkt[:, cs] = jnp.zeros((D, TQ), f32)
        dvt[:, cs] = jnp.zeros((D, TQ), f32)
        return carry

    jax.lax.fori_loop(0, ZB, zero_blk, 0)
    qkv_copies[2].start()
    x_copy(1).start()
    jax.lax.fori_loop(ZB, NB, zero_blk, 0)

    def ln_block(b):
        r0 = pl.multiple_of(b * TQ, TQ)
        xn, _ = _layernorm(x_v[pl.ds(r0, TQ), :].astype(f32))
        xnt[:, pl.ds(r0, TQ)] = _pk(xn.T)
        return _pk(xn)

    def proj_block(b, first):
        r0 = pl.multiple_of(b * TQ, TQ)
        r2 = pl.multiple_of(b * (TQ // 2), TQ // 2)
        xb = _upk(hn_b[...])

        def finish(y, nat, tr):
            y_t = y.astype(bf16).astype(f32).T
            tr[:, pl.ds(r0, TQ)] = y_t
            y_p = jnp.concatenate([y_t, jnp.zeros((48, TQ), f32)], axis=0)
            for g in range(NG):
                c0 = HG * DH * g
                nat[_prow(g, r2, TQ // 2), :] = _pk(y_p[c0:c0 + 128].T)

        if first:
            qkv_copies[1].wait()
            qkv_copies[0].start()
        k = _dot(xb, wqkv_v[:, D:2 * D])
        if first:
            qkv_copies[2].wait()
            x_copy(1).wait()
            v = _dot(xb, wqkv_v[:, 2 * D:3 * D])
            finish(k, knat, kt)
            for bb in range(2, NB):
                x_copy(bb).start()
            qkv_copies[0].wait()
            q = _dot(xb, wqkv_v[:, 0:D]) * QSCALE
            xb_next = ln_block(1)
            finish(v, vnat, vt)
        else:
            xb_next = ln_block(jnp.minimum(b + 1, NB - 1))
            finish(k, knat, kt)
            finish(_dot(xb, wqkv_v[:, 2 * D:3 * D]), vnat, vt)
            q = _dot(xb, wqkv_v[:, 0:D]) * QSCALE
        qt[b] = q.T
        hn_b[...] = xb_next

    def phase0():
        x_copy(0).wait()
        hn_b[...] = ln_block(0)
        proj_block(0, True)
        for cp in in_copies:
            cp.start()

        def blk(b, carry):
            @pl.when(b + 1 < NB)
            def _():
                x_copy(b + 1).wait()

            proj_block(b, False)
            return carry

        jax.lax.fori_loop(1, NB, blk, 0)

    phase0()

    for cp in in_copies:
        cp.wait()

    def main():
        ot[...] = jnp.zeros_like(ot)
        dqb[...] = jnp.zeros_like(dqb)
        sbuf = (s_a, s_b)
        HC = NCK // NS

        def save_dq(b):
            dqt[pl.ds(pl.multiple_of(b * (D // 2), 8), D // 2), :] = _pk(dqb[...])

        def score_weights(qn, h0, k):
            rs, off = _head_window(h0, k)
            win = jnp.where(_row_mask(24, off), qt[qn, rs, :], 0.0)
            return _group(h0, k), _group_weights(win, k)

        def score_chunk(g, w, c, dst, m):
            for s0 in range(0, CK, SUB):
                r = c * CK + s0
                s = _dot(_upk(knat[_prow(g, r // 2, SUB // 2), :]), w)
                dst[c // HC][pl.ds((c % HC) * CK + s0, SUB), :] = s
                mc = jnp.max(s.reshape(SUB // 8, 8, TQ), axis=0)
                m = mc if m is None else jnp.maximum(m, mc)
            return m

        g0, w0 = score_weights(0, 0, 0)
        m0 = None
        for c in range(NCK):
            m0 = score_chunk(g0, w0, c, sbuf[0], m0)
        m_v[...] = jnp.broadcast_to(jnp.max(m0, axis=0, keepdims=True), (8, TQ))
        da_v[0] = _dot_nt(gy_v[0:TQ, :], wd_v[0])

        def qblock(qb, carry):
            r0 = pl.multiple_of(qb * TQ, TQ)
            z = jax.lax.shift_right_logical(qb, 20) * 8
            later = qb > 0

            def acc(old, new):
                return jnp.where(later, old, 0.0) + new

            def fwd_iter(i, carry2):
                h0 = HPF * i
                wrap = jax.lax.shift_right_logical(h0 + HPF, 5)
                nxt = [(qb, h0, k + 1) for k in range(HPF - 1)]
                nxt.append((jnp.minimum(qb + wrap, NB - 1), jnp.bitwise_and(h0 + HPF, H - 1), 0))
                mrow = [m_v[0:1, :]]
                rows = jax.lax.broadcasted_iota(jnp.int32, (24, CK), 0)
                n_steps = HPF * NCK
                m = o = gw = None
                for n in range(n_steps + LAG):
                    if n < n_steps:
                        k, c = divmod(n, NCK)
                        if c == 0:
                            gw = score_weights(*nxt[k])
                            m = None
                        m = score_chunk(gw[0], gw[1], c, sbuf[(k + 1) % 2], m)
                        if c == NCK - 1:
                            mrow.append(jnp.max(m, axis=0, keepdims=True))
                    if n >= LAG:
                        k, c = divmod(n - LAG, NCK)
                        rs, off = _head_window(h0, k)
                        one = 23 if off == 0 else 0
                        src = sbuf[k % 2][c // HC]
                        sv = src[pl.ds(pl.multiple_of(z + (c % HC) * CK, 8), CK), :]
                        p = jnp.exp2(sv - mrow[k]).astype(bf16)
                        p_refs[c][_pslot(h0, k), :] = pltpu.bitcast(p, u32)
                        vl = jnp.where(rows == one, 1.0, vt[rs, pl.ds(c * CK, CK)])
                        oc = _dot(vl, p)
                        o = oc if c == 0 else o + oc
                        if c == NCK - 1:
                            li = 1.0 / o[one:one + 1]
                            linv[h0 + k] = jnp.broadcast_to(li, (8, TQ))
                            ot[rs, :] = jnp.where(_row_mask(24, off), o * li, ot[rs, :])
                m_v[...] = jnp.broadcast_to(mrow[-1], (8, TQ))
                return carry2

            jax.lax.fori_loop(0, H // HPF, fwd_iter, 0)

            gyb = gy_v[pl.ds(r0, TQ), :]
            da_v[1] = _dot_nt(gyb, wd_v[1])
            save_dq(jnp.maximum(qb - 1, 0))
            o_t = ot[...]
            otb[...] = _pk(o_t)
            attn = _dot(o_t.T.astype(bf16), wo_v[...])
            dhn_acc[...] = jnp.zeros_like(dhn_acc)
            hres = x_v[pl.ds(r0, TQ), :].astype(f32) + attn
            y_acc[...] = hres
            hn, rstd = _layernorm(hres)
            hn_f[...] = hn
            rstd_v[...] = rstd
            hn_b[...] = _pk(hn)
            hnt[...] = _pk(hn.T)
            for c in range(2, NFC):
                da_v[c] = _dot_nt(gyb, wd_v[c])

            def ffn_a(c):
                hb = _upk(hn_b[...])
                g = _dot(hb, wg_v[c])
                u = _dot(hb, wu_v[c])
                return g, u

            def ffn_b(c, g, u):
                da = da_v[c]
                g2 = g * g
                t = jnp.tanh(GELU_C * g * (1.0 + GELU_A * g2))
                hg = 0.5 * g
                gel = hg + hg * t
                dgel = 0.5 + 0.5 * t + hg * (1.0 - t * t) * (GELU_C + 3.0 * GELU_A * GELU_C * g2)
                af = gel * u
                a = af.astype(bf16)
                dg = (da * u * dgel).astype(bf16)
                du = (da * gel).astype(bf16)
                y_acc[...] += _dot(a, wd_v[c])
                dhn_acc[...] += _dot_nt(dg, wg_v[c]) + _dot_nt(du, wu_v[c])
                ht = _upk(hnt[...])
                a_wg[c] = acc(a_wg[c], _dot(ht, dg))
                a_wu[c] = acc(a_wu[c], _dot(ht, du))
                a_wd[c] = acc(a_wd[c], _dot(af.T, gy_v[pl.ds(r0, TQ), :]))

            def ffn_pair(i, c):
                r_0 = ffn_a(2 * i)
                r_1 = ffn_a(2 * i + 1)
                ffn_b(2 * i, *r_0)
                ffn_b(2 * i + 1, *r_1)
                return c

            jax.lax.fori_loop(0, NFC // 2, ffn_pair, 0)

            rn = pl.multiple_of(jnp.minimum(qb + 1, NB - 1) * TQ, TQ)
            da_v[0] = _dot_nt(gy_v[pl.ds(rn, TQ), :], wd_v[0])

            h2_v[pl.ds(r0, TQ), :] = y_acc[...].astype(bf16)
            dh = gy_v[pl.ds(r0, TQ), :].astype(f32) + _layernorm_bwd(
                dhn_acc[...], hn_f[...], rstd_v[...])
            dh_v[pl.ds(r0, TQ), :] = dh
            dhb = dh.astype(bf16)
            dot_[...] = _dot_nt(wo_v[...], dhb)
            a_wo[...] = acc(a_wo[...], _dot(_upk(otb[...]), dhb))

            def head_terms(h0, k):
                rs, off = _head_window(h0, k)
                m24 = _row_mask(24, off)
                do_l = jnp.where(m24, dot_[rs, :] * linv[h0 + k][0:1, :], 0.0)
                delta = jnp.sum(do_l * ot[rs, :], axis=0, keepdims=True)
                return h0, k, _group_weights(do_l, k), rs, m24, do_l, delta

            def ds_chunk(t, c):
                h0, k, w, _, _, _, delta = t
                parts = []
                for s0 in range(0, CK, SUB):
                    r = c * CK + s0
                    parts.append(
                        _dot(_upk(vnat[_prow(_group(h0, k), r // 2, SUB // 2), :]), w))
                dp = jnp.concatenate(parts, axis=0)
                p = _upk(p_refs[c][_pslot(h0, k), :])
                return (p.astype(f32) * (dp - delta)).astype(bf16)

            ds0[...] = pltpu.bitcast(ds_chunk(head_terms(0, 0), 0), u32)
            pltpu.make_async_copy(h2_v.at[pl.ds(r0, TQ), :], h2_hbm.at[pl.ds(r0, TQ), :],
                                  sem_h2.at[qb]).start()

            def bwd_iter(i, carry2):
                h0 = HPB * i
                terms = [head_terms(h0, k) for k in range(HPB)]
                terms.append(head_terms(jnp.minimum(h0 + HPB, H - HPB), 0))
                ds = _upk(ds0[...])
                dq = None
                for n in range(HPB * NCK):
                    k, c = divmod(n, NCK)
                    _, _, _, rs, m24, do_l, _ = terms[k]
                    if c == 0:
                        q_l = jnp.where(m24, qt[qb, rs, :], 0.0)
                    kn, cn = divmod(n + 1, NCK)
                    ds_next = ds_chunk(terms[kn], cn)
                    sl = pl.ds(c * CK, CK)
                    p = _upk(p_refs[c][_pslot(h0, k, z), :])
                    dvt[rs, sl] += _dot_nt(do_l, p)
                    dkt[rs, sl] += _dot_nt(q_l, ds)
                    dqc = _dot(kt[rs, sl], ds)
                    dq = dqc if c == 0 else dq + dqc
                    if c == NCK - 1:
                        dqb[rs, :] = jnp.where(m24, dq * SCALE, dqb[rs, :])
                    ds = ds_next
                ds0[...] = pltpu.bitcast(ds, u32)
                return carry2

            jax.lax.fori_loop(0, H // HPB, bwd_iter, 0)
            return carry

        jax.lax.fori_loop(0, NB, qblock, 0)
        save_dq(NB - 1)

    main()

    w_copies = [pltpu.make_async_copy(wo_v, dwo_hbm, sem_w.at[0])]
    for c in range(NFC):
        cs = pl.ds(c * FC, FC)
        w_copies += [pltpu.make_async_copy(wg_v.at[c], dwg_hbm.at[:, cs], sem_w.at[1 + 3 * c]),
                     pltpu.make_async_copy(wu_v.at[c], dwu_hbm.at[:, cs], sem_w.at[2 + 3 * c]),
                     pltpu.make_async_copy(wd_v.at[c], dwd_hbm.at[cs, :], sem_w.at[3 + 3 * c])]

    RW = D // NB

    def blk_a(b, carry):
        cs = pl.ds(pl.multiple_of(b * TQ, TQ), TQ)
        rd = pl.ds(pl.multiple_of(b * (D // 2), 8), D // 2)
        dq_p = dqt[rd, :]
        dk_b = (dkt[:, cs] * LN2).astype(bf16)
        dv_b = dvt[:, cs].astype(bf16)
        for m0 in range(0, D, MS):
            ms = slice(m0, m0 + MS)
            qt[b, ms, :] = (_dot(wqkv_v[ms, 0:D], _upk(dq_p)) + _dot(wqkv_v[ms, D:2 * D], dk_b)
                            + _dot(wqkv_v[ms, 2 * D:3 * D], dv_b))
        p_refs[0][rd, :] = pltpu.bitcast(dk_b, u32)
        p_refs[1][rd, :] = pltpu.bitcast(dv_b, u32)
        ra = pl.ds(pl.multiple_of(b * RW, 16), RW)
        rb = pl.ds(pl.multiple_of(b * (FC // NB), 16), FC // NB)
        wo_v[ra, :] = a_wo[ra, :].astype(bf16)
        for c in range(NFC):
            wg_v[c, ra, :] = a_wg[c, ra, :].astype(bf16)
            wu_v[c, ra, :] = a_wu[c, ra, :].astype(bf16)
            wd_v[c, rb, :] = a_wd[c, rb, :].astype(bf16)
        return carry

    jax.lax.fori_loop(0, NB, blk_a, 0)
    for cp in w_copies:
        cp.start()

    def blk_b(b, carry):
        cs = pl.ds(pl.multiple_of(b * TQ, TQ), TQ)
        ra = pl.ds(pl.multiple_of(b * RW, 16), RW)
        xr = pl.ds(pl.multiple_of(b * (RW // 2), 8), RW // 2)
        xn, rstd = _layernorm(x_v[cs, :].astype(f32))
        dx = dh_v[cs, :] + _layernorm_bwd(qt[b].T, xn, rstd)
        gy_v[cs, :] = dx.astype(bf16)
        for j, src in enumerate((dqt, p_refs[0], p_refs[1])):
            for n in range(D // WC):
                acc_w = None
                for t in range(NB):
                    r = t * (D // 2) + n * (WC // 2)
                    part = _dot_nt(_upk(xnt[xr, t * TQ:(t + 1) * TQ]), _upk(src[r:r + WC // 2, :]))
                    acc_w = part if acc_w is None else acc_w + part
                wqkv_v[ra, j * D + n * WC:j * D + (n + 1) * WC] = acc_w.astype(bf16)
        pltpu.make_async_copy(gy_v.at[cs, :], dx_hbm.at[cs, :], sem_dx.at[b]).start()
        pltpu.make_async_copy(wqkv_v.at[ra, :], dwqkv_hbm.at[ra, :], sem_wq.at[b]).start()
        return carry

    jax.lax.fori_loop(0, NB, blk_b, 0)

    for b in range(NB):
        rs = pl.ds(b * TQ, TQ)
        pltpu.make_async_copy(h2_v.at[rs, :], h2_hbm.at[rs, :], sem_h2.at[b]).wait()
    for cp in w_copies:
        cp.wait()
    for b in range(NB):
        rs = pl.ds(b * TQ, TQ)
        ra = pl.ds(b * RW, RW)
        pltpu.make_async_copy(gy_v.at[rs, :], dx_hbm.at[rs, :], sem_dx.at[b]).wait()
        pltpu.make_async_copy(wqkv_v.at[ra, :], dwqkv_hbm.at[ra, :], sem_wq.at[b]).wait()


@jax.jit
def pallas_sequential_preLN__softmax_full_mha__glu_gated_geglu__prompt_kernel(
    A_x: jax.Array,
    A_wqkv: jax.Array,
    A_wo: jax.Array,
    B_x: jax.Array,
    B_w_gate: jax.Array,
    B_w_up: jax.Array,
    B_w_down: jax.Array,
    grad_out: jax.Array,
):
    del B_x
    any_spec = pl.BlockSpec(memory_space=pl.ANY)
    out_shape = (
        jax.ShapeDtypeStruct((S, D), bf16),
        jax.ShapeDtypeStruct((S, D), bf16),
        jax.ShapeDtypeStruct((D, 3 * D), bf16),
        jax.ShapeDtypeStruct((D, D), bf16),
        jax.ShapeDtypeStruct((D, DF), bf16),
        jax.ShapeDtypeStruct((D, DF), bf16),
        jax.ShapeDtypeStruct((DF, D), bf16),
    )
    scratch = [
        pltpu.VMEM((S, D), bf16),
        pltpu.VMEM((S, D), bf16),
        pltpu.VMEM((D, 3 * D), bf16),
        pltpu.VMEM((D, D), bf16),
        pltpu.VMEM((NFC, D, FC), bf16),
        pltpu.VMEM((NFC, D, FC), bf16),
        pltpu.VMEM((NFC, FC, D), bf16),
        pltpu.VMEM((S, D), bf16),
        pltpu.VMEM((NB, D, TQ), f32),
        pltpu.VMEM((NG * S // 2, 128), u32),
        pltpu.VMEM((NG * S // 2, 128), u32),
        pltpu.VMEM((D, S), f32),
        pltpu.VMEM((D, S), f32),
        pltpu.VMEM((D // 2, S), u32),
        pltpu.VMEM((D, S), f32),
        pltpu.VMEM((D, S), f32),
        pltpu.VMEM((NB * D // 2, TQ), u32),
        pltpu.VMEM((S, D), f32),
        pltpu.VMEM((NFC, D, FC), f32),
        pltpu.VMEM((NFC, D, FC), f32),
        pltpu.VMEM((NFC, FC, D), f32),
        pltpu.VMEM((D, D), f32),
        [pltpu.VMEM((H * CK // 2, TQ), u32)] * NCK,
        [pltpu.VMEM((S // NS, TQ), f32)] * NS,
        [pltpu.VMEM((S // NS, TQ), f32)] * NS,
        pltpu.VMEM((8, TQ), f32),
        pltpu.VMEM((D, TQ), f32),
        pltpu.VMEM((D, TQ), f32),
        pltpu.VMEM((D, TQ), f32),
        pltpu.VMEM((H, 8, TQ), f32),
        pltpu.VMEM((TQ, D), f32),
        pltpu.VMEM((TQ // 2, D), u32),
        pltpu.VMEM((D // 2, TQ), u32),
        pltpu.VMEM((D // 2, TQ), u32),
        pltpu.VMEM((TQ, D), f32),
        pltpu.VMEM((TQ, D), f32),
        pltpu.VMEM((TQ, 1), f32),
        pltpu.VMEM((NFC, TQ, FC), f32),
        pltpu.VMEM((CK // 2, TQ), u32),
        pltpu.SemaphoreType.DMA((NB,)),
        pltpu.SemaphoreType.DMA((3,)),
        pltpu.SemaphoreType.DMA((2 + 3 * NFC,)),
        pltpu.SemaphoreType.DMA((NB,)),
        pltpu.SemaphoreType.DMA((NB,)),
        pltpu.SemaphoreType.DMA((1 + 3 * NFC,)),
        pltpu.SemaphoreType.DMA((NB,)),
    ]
    outs = pl.pallas_call(
        _kernel,
        out_shape=out_shape,
        in_specs=[any_spec] * 7,
        out_specs=[any_spec] * 7,
        scratch_shapes=scratch,
        compiler_params=pltpu.CompilerParams(vmem_limit_bytes=124 * 1024 * 1024),
    )(A_x.reshape(S, D), A_wqkv, A_wo, B_w_gate, B_w_up, B_w_down, grad_out.reshape(S, D))
    h2, dx, dwqkv, dwo, dwg, dwu, dwd = outs
    return (h2.reshape(1, S, D), dx.reshape(1, S, D), dwqkv, dwo, dwg, dwu, dwd)
```
